```python
import os as _os
_os.environ.setdefault('JAX_PLATFORMS', 'cpu')
import jax
import jax.numpy as jnp

def _softmax(x, axis=-1):
    return jax.nn.softmax(x, axis=axis)

def _gelu(x):
    return jax.nn.gelu(x, approximate=True)

def _silu(x):
    return jax.nn.silu(x)

def _sigmoid(x):
    return jax.nn.sigmoid(x)

def _layernorm(x, axis=-1, eps=1e-05):
    m = jnp.mean(x, axis=axis, keepdims=True)
    v = jnp.var(x, axis=axis, keepdims=True)
    return (x - m) / jnp.sqrt(v + eps)

def _scatter_add(tgt, idx, src, axis=0):
    return tgt.at[idx].add(src)

def _segment_sum(src, seg, n):
    return jax.ops.segment_sum(src, seg, n)

class _Rng:

    def __init__(self, key):
        self._k = key

    def _next(self):
        self._k, sub = jax.random.split(self._k)
        return sub

    def normal(self, shape):
        return jax.random.normal(self._next(), shape, dtype=jnp.bfloat16)

    def randint(self, lo, hi, shape):
        return jax.random.randint(self._next(), shape, lo, hi, dtype=jnp.int32)

    def uniform(self, shape, lo=0.0, hi=1.0):
        return jax.random.uniform(self._next(), shape, jnp.bfloat16, lo, hi)

    def permutation(self, n):
        return jax.random.permutation(self._next(), n)
kernel_name = 'concat_heads__linear_kernel_hedgehog__memory_aug_recurrent_mem_tr__prompt'

def setup_inputs():
    _rng = _Rng(jax.random.key(int.from_bytes(__import__("os").urandom(4), "little")))
    _w = lambda a: (lambda t: t.astype(jnp.bfloat16) if jnp.issubdtype(t.dtype, jnp.floating) else t)(jnp.asarray(a))

    def _A_setup():
        B, S, D, H = (1, 2048, 576, 32)
        Dh = D // H
        return {'x': _w((lambda *s: _rng.normal(s) * 0.4)(B, S, D)), 'wqkv': _w((lambda *s: _rng.normal(s) * 0.4)(D, 3 * D)), 'w_phi': _w((lambda *s: _rng.normal(s) * 0.4)(H, Dh, Dh) * Dh ** (-0.5)), 'wo': _w((lambda *s: _rng.normal(s) * 0.05)(D, D))}
    _A_in = _A_setup()

    def _B_setup():
        B, S, Dm = (1, 2048, 576)
        H, Dh = (32, 128)
        M, seg = (8, 32)
        seg = min(seg, S)
        S = S // seg * seg
        return {'x': _w((lambda *s: _rng.normal(s) * 0.05)(B, S, Dm)), 'mem0': _w((lambda *s: _rng.normal(s) * 0.8)(B, M, Dm)), 'Wq': _w((lambda *s: _rng.normal(s) * 3.2)(Dm, H, Dh) * Dm ** (-0.5)), 'Wk': _w((lambda *s: _rng.normal(s) * 3.2)(Dm, H, Dh) * Dm ** (-0.5)), 'Wv': _w((lambda *s: _rng.normal(s) * 0.8)(Dm, H, Dh) * Dm ** (-0.5)), 'Wo': _w((lambda *s: _rng.normal(s) * 0.8)(H, Dh, Dm) * (H * Dh) ** (-0.5)), 'seg_len': seg}
    _B_in = _B_setup()
    return {'A_x': _A_in['x'], 'A_wqkv': _A_in['wqkv'], 'A_w_phi': _A_in['w_phi'], 'A_wo': _A_in['wo'], 'B_x': _B_in['x'], 'B_mem0': _B_in['mem0'], 'B_Wq': _B_in['Wq'], 'B_Wk': _B_in['Wk'], 'B_Wv': _B_in['Wv'], 'B_Wo': _B_in['Wo'], 'B_seg_len': _B_in['seg_len']}

def reference(A_x, A_wqkv, A_w_phi, A_wo, B_x, B_mem0, B_Wq, B_Wk, B_Wv, B_Wo, B_seg_len):

    def _A_ref(x, wqkv, w_phi, wo):
        B, S, D = x.shape
        H = 32
        Dh = D // H
        qkv = (lambda x, *d: x.transpose(*d))((x @ wqkv).reshape(B, S, 3, H, Dh), 2, 0, 3, 1, 4)
        q, k, v = (qkv[0], qkv[1], qkv[2])
        pq = jnp.einsum('bhsd,hdf->bhsf', q, w_phi)
        pk = jnp.einsum('bhsd,hdf->bhsf', k, w_phi)
        phi_q = jnp.concatenate([_softmax(pq, axis=-1), _softmax(-pq, axis=-1)], axis=-1)
        phi_k = jnp.concatenate([_softmax(pk, axis=-1), _softmax(-pk, axis=-1)], axis=-1)
        kv = jnp.einsum('bhsf,bhsd->bhfd', phi_k, v)
        z = jnp.einsum('bhsf->bhf', phi_k)
        num = jnp.einsum('bhqf,bhfd->bhqd', phi_q, kv)
        den = jnp.einsum('bhqf,bhf->bhq', phi_q, z)[..., None] + 1e-06
        o = num / den
        return (lambda x, *d: x.transpose(*d))(o, 0, 2, 1, 3).reshape(B, S, D) @ wo

    def _B_ref(x, mem0, Wq, Wk, Wv, Wo, seg_len):
        B, S, Dm = x.shape
        H, Dh = (Wq.shape[1], Wq.shape[2])
        M = mem0.shape[1]
        scale = Dh ** (-0.5)
        n_seg = S // seg_len
        L = M + seg_len
        idx = jnp.arange(L)
        mask = (idx[:, None] < M) | (idx[:, None] >= idx[None, :])
        mem = mem0
        outs = []
        for s in range(n_seg):
            xs = x[:, s * seg_len:(s + 1) * seg_len, :].copy()
            h = jnp.concatenate([mem, xs], axis=1)
            q = jnp.einsum('btd,dhe->bhte', h, Wq)
            k = jnp.einsum('btd,dhe->bhte', h, Wk)
            v = jnp.einsum('btd,dhe->bhte', h, Wv)
            scores = jnp.einsum('bhqe,bhke->bhqk', q, k) * scale
            scores = jnp.where(mask[None, None], scores, -1000000000.0)
            p = _softmax(scores, axis=-1)
            o = jnp.einsum('bhqk,bhke->bhqe', p, v)
            o = jnp.einsum('bhte,hed->btd', o, Wo)
            mem = o[:, :M, :].copy()
            outs.append(o[:, M:, :])
        return jnp.concatenate(outs, axis=1)
    a = _A_ref(A_x, A_wqkv, A_w_phi, A_wo)
    b = _B_ref(B_x, B_mem0, B_Wq, B_Wk, B_Wv, B_Wo, B_seg_len)
    return jnp.concatenate([a, b], axis=-1)
```

```python
import functools
import jax
import jax.numpy as jnp
from jax import lax
from jax.experimental import pallas as pl
from jax.experimental.pallas import tpu as pltpu

f32, bf16, u32, i32 = jnp.float32, jnp.bfloat16, jnp.uint32, jnp.int32

S, DM = 2048, 576
H, E, M, SEG = 32, 128, 8, 32
NP = H // 2
NPER = S // (4 * SEG)
AH, AD = 32, 18
G, GR = 4, 144
SCALE = float(E) ** -0.5
LOG2E = 1.4426950408889634


def _dot(a, b):
    return jnp.dot(a, b, preferred_element_type=f32)


def _dot_nt(a, b):
    return lax.dot_general(a, b, (((1,), (1,)), ((), ())), preferred_element_type=f32)


def _b(x):
    return pltpu.bitcast(x, bf16)


def _u(x):
    return pltpu.bitcast(x, u32)


def _iota(shape, dim):
    return lax.broadcasted_iota(i32, shape, dim)


def _features(p):
    x3 = p.reshape(AD, 8, 128)
    mx = jnp.max(x3, axis=0)
    mn = jnp.min(x3, axis=0)
    ep = jnp.exp(x3 - mx[None])
    en = jnp.exp(mn[None] - x3)
    rp = 1.0 / jnp.sum(ep, axis=0)
    rn = 1.0 / jnp.sum(en, axis=0)
    phi = jnp.concatenate([ep * rp[None], en * rn[None]], axis=0)
    return phi.reshape(2 * GR, 128).astype(bf16)


def _kernel(xat_h, wa_h, phi_h, woa_h, xbt_h, mem_h, wq_h, wk_h, wv_h, wot_h, out_h,
            xat, wa, phi, woa, xbt, mem0, wst, wot,
            pc, wkv, wqt, wop, kvacc, kvt,
            wqkv, wo32, xnat, A0, A1, ringB, odef, fill, outb,
            sem_in, sem_w, sem_out, *, nper):
    cps = [
        pltpu.make_async_copy(wa_h, wa, sem_in.at[0]),
        pltpu.make_async_copy(phi_h, phi, sem_in.at[1]),
        pltpu.make_async_copy(xat_h, xat, sem_in.at[2]),
        pltpu.make_async_copy(xbt_h, xbt, sem_in.at[3]),
        pltpu.make_async_copy(mem_h, mem0, sem_in.at[4]),
        pltpu.make_async_copy(woa_h, woa, sem_in.at[5]),
        pltpu.make_async_copy(wot_h, wot, sem_in.at[6]),
    ]
    wcp = [pltpu.make_async_copy(w, wst.at[i], sem_w.at[i]) for i, w in enumerate((wq_h, wk_h, wv_h))]
    for c in cps[:3]:
        c.start()
    for c in wcp:
        c.start()
    for c in cps[3:]:
        c.start()

    cps[0].wait()
    cps[1].wait()
    pc[...] = jnp.zeros_like(pc)
    for d in range(AD):
        pc[0:AD, 32 * d:32 * d + 32] = phi[d].astype(f32)
    row = _iota((DM, 640), 0)
    col = _iota((DM, 640), 1)
    perm = jnp.where(col == (row & 31) * AD + (row >> 5), 1.0, 0.0).astype(bf16)
    rt = _dot(pc[:, 0:DM].astype(bf16), perm)
    rtk = pltpu.roll(rt, 64, 1)
    r2 = _iota((GR, 256), 0)
    c2 = _iota((GR, 256), 1)

    def bdt(src, g, shift):
        w = src[0:AD, 128 * g:128 * g + 256]
        w = jnp.broadcast_to(w[:, None, :], (AD, 8, 256)).reshape(GR, 256)
        rel = c2 + (128 * g - shift - GR * g) - (r2 & 7) * AD
        return jnp.where((rel >= 0) & (rel < AD), w, 0.0).astype(bf16)

    def prep_kv():
        for g in range(G):
            wk_g = _dot_nt(bdt(rtk, g, 64), wa[:, 512 + 128 * g:512 + 128 * g + 256])
            wkv[GR * g:GR * g + 72, :] = _u(wk_g.astype(bf16))
            pv = jnp.where(c2 + (128 * g - GR * g) == (r2 & 7) * AD + (r2 >> 3), 1.0, 0.0).astype(bf16)
            kw = 256 if g < 3 else 192
            wv_g = _dot_nt(pv[:, :kw], wa[:, 1152 + 128 * g:1152 + 128 * g + kw])
            wkv[GR * g + 72:GR * g + 144, :] = _u(wv_g.astype(bf16))

    def prep_q():
        for g in range(G):
            wq_g = _dot_nt(bdt(rt, g, 0), wa[:, 128 * g:128 * g + 256])
            wqt[72 * g:72 * g + 72, :] = _u(wq_g.astype(bf16))

    def prep_wo():
        r3 = _iota((GR, GR), 0)
        c3 = _iota((GR, GR), 1)
        pw = jnp.where(c3 == (r3 & 7) * AD + (r3 >> 3), 1.0, 0.0).astype(bf16)
        for g in range(G):
            wop[72 * g:72 * g + 72, :] = _u(_dot(pw, woa[GR * g:GR * g + GR, :]).astype(bf16))

    prep_kv()
    prep_q()

    cps[2].wait()
    kvacc[...] = jnp.zeros_like(kvacc)
    ones_pad = jnp.where(_iota((16, 128), 0) < 8, 1.0, 0.0).astype(f32)

    def a1(c, carry):
        xt = xat[:, pl.ds(pl.multiple_of(c * 128, 128), 128)]
        for g in range(G):
            y = _dot(_b(wkv[GR * g:GR * g + GR, :]), xt)
            ph = _features(y[0:GR])
            va = jnp.concatenate([y[GR:2 * GR], ones_pad], axis=0).astype(bf16)
            kvacc[g] += _dot_nt(va, ph)
        return carry
    lax.fori_loop(0, S // 128, a1, 0)
    r4 = _iota((160, 288), 0)
    c4 = _iota((160, 288), 1)
    for g in range(G):
        kvt[g] = _u(jnp.where((r4 & 7) == (c4 & 7), kvacc[g], 0.0).astype(bf16))
    cps[5].wait()
    prep_wo()

    for which in range(3):
        wcp[which].wait()
        w32 = wst.at[which].bitcast(u32)

        def body(i, c, w32=w32, which=which):
            sub = w32.at[pl.ds(pl.multiple_of(i * 256, 256), 256), :]
            r = pl.multiple_of(i * 8, 8)
            for j in range(16):
                ev = sub[pl.ds(j, 8, stride=32), :]
                od = sub[pl.ds(j + 16, 8, stride=32), :]
                lo = (ev & u32(0xFFFF)) | (od << 16)
                hi = (ev >> 16) | (od & u32(0xFFFF0000))
                c0 = (2 * j) * 384 + which * 128
                wqkv[pl.ds(r, 8), c0:c0 + 128] = lo
                wqkv[pl.ds(r, 8), c0 + 384:c0 + 512] = hi
            return c
        lax.fori_loop(0, DM // 16, body, 0)

    cps[6].wait()

    def two(h, c):
        blk = wot[pl.ds(pl.multiple_of(h * DM, 16), DM), :]
        wo32[pl.ds(pl.multiple_of(h * 64, 64), 64), :] = _u(blk.T)
        return c
    lax.fori_loop(0, H, two, 0)

    cps[3].wait()
    cps[4].wait()

    def xtrans(gidx):
        c0 = pl.multiple_of(gidx * 128, 128)
        xnat[pl.ds(c0, 128), :] = xbt[:, pl.ds(c0, 128)].astype(f32).T
    xtrans(0)
    xtrans(1)

    odef[...] = jnp.zeros_like(odef)
    ri = _iota((80, 80), 0)
    ci = _iota((80, 80), 1)
    same = (ri < 40) == (ci < 40)
    valid = same & (((ri >= 32) & (ri < 48)) | ((ci >= 32) & (ci < 48)) | (ci <= ri))
    fill[...] = jnp.where(valid, 0.0, jnp.where(same, -1e9 / SCALE, -jnp.inf)).astype(f32)

    def W(c0, n):
        return _b(wqkv[:, pl.ds(c0, n)])

    def WO(r0, n):
        return _b(wo32[r0 // 2:(r0 + n) // 2, :])

    def tails(p):
        return jnp.concatenate(
            [xnat[pl.ds(pl.multiple_of(128 * p + 32 * c + 24, 8), 8), :] for c in range(4)], axis=0)

    lhs0 = jnp.concatenate([tails(0), xnat[0:32, :]], axis=0).astype(bf16)

    def pro(i, c):
        c0 = pl.multiple_of(i * 768, 128)
        y = _dot(lhs0, W(c0, 768))
        ringB[0, :, pl.ds(c0, 768)] = y[0:32]
        A0[0:24, pl.ds(c0, 768)] = y[32:56]
        return c
    lax.fori_loop(0, NP, pro, 0)

    def out_copy(gidx):
        r0 = pl.multiple_of(gidx * 128, 128)
        return pltpu.make_async_copy(outb.at[pl.ds(r0, 128), :], out_h.at[pl.ds(r0, 128), :], sem_out.at[gidx])

    def period(p, mem):
        pn = jnp.minimum(p + 1, NPER - 1)
        pp = jnp.maximum(p - 1, 0)
        pcur = p % 2
        pnx = 1 - pcur
        xo = tails(pn).astype(bf16)
        xt = xat[:, pl.ds(pl.multiple_of(p * 128, 128), 128)]
        st = {"oacc": None}

        def a2_pq():
            st["ph"] = [_features(_dot(_b(wqt[72 * g:72 * g + 72, :]), xt)) for g in range(G)]

        def a2_num():
            os_ = []
            for g in range(G):
                nd = _dot(_b(kvt[g]), st["ph"][g])
                rden = 1.0 / (nd[GR:GR + 8] + 1e-6)
                os_.append((nd[0:GR].reshape(AD, 8, 128) * rden[None]).reshape(GR, 128))
            st["oa"] = jnp.concatenate(os_, axis=0).T.astype(bf16)

        def a2_out():
            y = _dot(st["oa"], _b(wop[...]))
            outb[pl.ds(pl.multiple_of(p * 128, 128), 128), 0:DM] = y.astype(bf16)

        a_stage = {0: a2_pq, 1: None, 2: a2_num, 3: a2_out}

        for r in range(4):
            Ac, An = (A0, A1) if r % 2 == 0 else (A1, A0)
            t = 4 * p + r
            tn = jnp.minimum(t + 1, 4 * NPER - 1)
            xn = xnat[pl.ds(pl.multiple_of(32 * tn, 32), 24), :]
            lhs = jnp.concatenate([mem, xn], axis=0).astype(bf16)
            fl = fill[...]
            Ac[24:32, :] = ringB[pcur, 8 * r:8 * r + 8, :]
            lo_def = odef[pnx, :, 1024 * r:1024 * r + 1024].astype(bf16)
            ys, ps, os_ = {}, {}, {}
            acc = [None]

            def st_qkv(i):
                y = _dot(lhs, W(768 * i, 768))
                An[0:24, 768 * i:768 * (i + 1)] = y[8:32]
                ys[i] = y[0:8]

            def gather(i, ym, o1):
                c1 = 768 * i + o1
                o2 = o1 + 384
                return jnp.concatenate([Ac[:, c1:c1 + 128], ym[:, o1:o1 + 128], ym[:, o2:o2 + 128],
                                        Ac[:, c1 + 384:c1 + 512]], axis=0).astype(bf16)

            def st_qk(i):
                s = _dot_nt(gather(i, ys[i], 0), gather(i, ys[i], 128))
                s = jnp.where(fl == 0.0, s, fl)
                m = jnp.max(s, axis=-1, keepdims=True)
                e = jnp.exp2((s - m) * (SCALE * LOG2E))
                ps[i] = (e.astype(bf16), jnp.sum(e, axis=-1, keepdims=True))

            def st_pv(i):
                e, l = ps.pop(i)
                os_[i] = _dot(e, gather(i, ys.pop(i), 256)) * (1.0 / l)

            def st_o(i):
                o = os_.pop(i)
                odef[pcur, 8 * r:8 * r + 8, 256 * i:256 * i + 128] = o[24:32]
                odef[pcur, 8 * r:8 * r + 8, 256 * i + 128:256 * i + 256] = o[72:80]
                l1 = jnp.concatenate([o[32:40], o[0:24]], axis=0)
                y = _dot(jnp.concatenate([l1, o[40:72]], axis=1).astype(bf16), WO(256 * i, 256))
                acc[0] = y if acc[0] is None else acc[0] + y

            def f_xqkv(j):
                c0 = r * 3072 + 768 * j
                ringB[pnx, :, c0:c0 + 768] = _dot(xo, W(c0, 768))

            def f_xo():
                y = _dot(lo_def, WO(1024 * r, 1024))
                st["oacc"] = y if st["oacc"] is None else st["oacc"] + y

            def f_a():
                if a_stage[r] is not None:
                    a_stage[r]()

            fillers = [[lambda: f_xqkv(0), f_a], [lambda: f_xqkv(1)], [lambda: f_xqkv(2), f_xo], [], [lambda: f_xqkv(3)]]
            for i in range(NP + 5):
                if i < NP:
                    st_qkv(i)
                else:
                    for f in fillers[i - NP]:
                        f()
                if 0 <= i - 1 < NP:
                    st_qk(i - 1)
                if 0 <= i - 2 < NP:
                    st_pv(i - 2)
                if 0 <= i - 3 < NP:
                    st_o(i - 3)
            outb[pl.ds(pl.multiple_of(32 * t, 32), 24), DM:2 * DM] = acc[0][8:32].astype(bf16)
            mem = acc[0][0:8]

        for c in range(4):
            outb[pl.ds(pl.multiple_of(128 * pp + 32 * c + 24, 8), 8), DM:2 * DM] = st["oacc"][8 * c:8 * c + 8].astype(bf16)
        xtrans(jnp.minimum(p + 2, NPER - 1))

        @pl.when(p > 0)
        def _():
            out_copy(pp).start()
        return mem

    lax.fori_loop(0, nper, period, mem0[...].astype(f32))
    y = _dot(odef[(nper - 1) % 2].astype(bf16), _b(wo32[...]))
    for c in range(4):
        outb[pl.ds(128 * (nper - 1) + 32 * c + 24, 8), DM:2 * DM] = y[8 * c:8 * c + 8].astype(bf16)
    out_copy(nper - 1).start()
    for gidx in range(nper):
        out_copy(gidx).wait()


def build(nper=NPER):
    V = pltpu.VMEM
    scratch = [
        V((DM, S), bf16),
        V((DM, 3 * DM), bf16),
        V((AD, AD, AH), bf16),
        V((DM, DM), bf16),
        V((DM, S), bf16),
        V((M, DM), bf16),
        V((3, DM * H, E), bf16),
        V((H * DM, E), bf16),
        V((32, 640), f32),
        V((DM, DM), u32),
        V((DM // 2, DM), u32),
        V((DM // 2, DM), u32),
        V((G, 160, 288), f32),
        V((G, 80, 288), u32),
        V((DM // 2, 3 * H * E), u32),
        V((H * E // 2, DM), u32),
        V((S, DM), f32),
        V((32, 3 * H * E), f32),
        V((32, 3 * H * E), f32),
        V((2, 32, 3 * H * E), f32),
        V((2, 32, H * E), f32),
        V((80, 80), f32),
        V((S, 2 * DM), bf16),
        pltpu.SemaphoreType.DMA((7,)),
        pltpu.SemaphoreType.DMA((3,)),
        pltpu.SemaphoreType.DMA((NPER,)),
    ]

    def fn(A_x, A_wqkv, A_w_phi, A_wo, B_x, B_mem0, B_Wq, B_Wk, B_Wv, B_Wo):
        out = pl.pallas_call(
            functools.partial(_kernel, nper=nper),
            out_shape=jax.ShapeDtypeStruct((S, 2 * DM), bf16),
            in_specs=[pl.BlockSpec(memory_space=pl.ANY)] * 10,
            out_specs=pl.BlockSpec(memory_space=pl.ANY),
            scratch_shapes=scratch,
            compiler_params=pltpu.CompilerParams(vmem_limit_bytes=112 * 1024 * 1024),
        )(
            jnp.swapaxes(A_x, 1, 2).reshape(DM, S),
            A_wqkv,
            jnp.transpose(A_w_phi, (1, 2, 0)),
            A_wo,
            jnp.swapaxes(B_x, 1, 2).reshape(DM, S),
            B_mem0.reshape(M, DM),
            B_Wq.reshape(DM * H, E),
            B_Wk.reshape(DM * H, E),
            B_Wv.reshape(DM * H, E),
            jnp.swapaxes(B_Wo, 1, 2).reshape(H * DM, E),
        )
        return out.reshape(1, S, 2 * DM)
    return fn


@functools.partial(jax.jit, static_argnames=("B_seg_len",))
def pallas_concat_heads__linear_kernel_hedgehog__memory_aug_recurrent_mem_tr__prompt_kernel(
    A_x, A_wqkv, A_w_phi, A_wo, B_x, B_mem0, B_Wq, B_Wk, B_Wv, B_Wo, B_seg_len,
):
    assert B_seg_len == SEG and A_x.shape == (1, S, DM) and B_x.shape == (1, S, DM)
    return build()(A_x, A_wqkv, A_w_phi, A_wo, B_x, B_mem0, B_Wq, B_Wk, B_Wv, B_Wo)
```

```python
import functools
import jax
import jax.numpy as jnp
from jax import lax
from jax.experimental import pallas as pl
from jax.experimental.pallas import tpu as pltpu

f32, bf16, u32, i32 = jnp.float32, jnp.bfloat16, jnp.uint32, jnp.int32

S, DM = 2048, 576
H, E, M, SEG = 32, 128, 8, 32
NP = H // 2
NPER = S // (4 * SEG)
AH, AD = 32, 18
G, GR = 4, 144
SCALE = float(E) ** -0.5
LOG2E = 1.4426950408889634


def _dot(a, b):
    return jnp.dot(a, b, preferred_element_type=f32)


def _dot_nt(a, b):
    return lax.dot_general(a, b, (((1,), (1,)), ((), ())), preferred_element_type=f32)


def _b(x):
    return pltpu.bitcast(x, bf16)


def _u(x):
    return pltpu.bitcast(x, u32)


def _iota(shape, dim):
    return lax.broadcasted_iota(i32, shape, dim)


def _features(p):
    t = p.shape[1]
    outs = []
    for g2 in range(2):
        x3 = p[72 * g2:72 * g2 + 72].reshape(9, 8, t)
        mx = jnp.max(x3, axis=0)
        mx = jnp.maximum(mx, pltpu.roll(mx, 4, 0))
        mn = jnp.min(x3, axis=0)
        mn = jnp.minimum(mn, pltpu.roll(mn, 4, 0))
        ep = jnp.exp(x3 - mx[None])
        en = jnp.exp(mn[None] - x3)
        sp = jnp.sum(ep, axis=0)
        sn = jnp.sum(en, axis=0)
        rp = 1.0 / (sp + pltpu.roll(sp, 4, 0))
        rn = 1.0 / (sn + pltpu.roll(sn, 4, 0))
        phi = jnp.concatenate([ep * rp[None], en * rn[None]], axis=0)
        outs.append(phi.reshape(GR, t).astype(bf16))
    return outs


def _kernel(xat_h, wa_h, phi_h, woa_h, xbt_h, mem_h, wq_h, wk_h, wv_h, wot_h, out_h,
            xat, wa, phi, woa, xbt, mem0, wst, wot,
            pc, wkv, wqt, wop, kvacc, kvt, pkb0, pkb1, vab0, vab1,
            wqkv, wo32, wor, xnat, A0, A1, ringB, odef, obuf, fill, outb,
            sem_in, sem_out, *, nper):
    xat_h, wa_h, woa_h, xbt_h, wot_h = [r.bitcast(u32) for r in (xat_h, wa_h, woa_h, xbt_h, wot_h)]
    cp_phi = pltpu.make_async_copy(phi_h, phi, sem_in.at[0])
    cp_wak = pltpu.make_async_copy(wa_h.at[:, 512:1152], wa.at[:, 512:1152], sem_in.at[1])
    cp_wav = pltpu.make_async_copy(wa_h.at[:, 1152:1728], wa.at[:, 1152:1728], sem_in.at[2])
    cp_waq = pltpu.make_async_copy(wa_h.at[:, 0:512], wa.at[:, 0:512], sem_in.at[3])
    cp_woa = pltpu.make_async_copy(woa_h, woa, sem_in.at[4])
    cp_mem = pltpu.make_async_copy(mem_h, mem0, sem_in.at[5])
    cp_xb0 = pltpu.make_async_copy(xbt_h.at[:, 0:384], xbt.at[:, 0:384], sem_in.at[6])
    cp_xb1 = pltpu.make_async_copy(xbt_h.at[:, 384:S], xbt.at[:, 384:S], sem_in.at[7])

    def cp_xa(c):
        cols = pl.ds(pl.multiple_of(c * 512, 512), 512)
        return pltpu.make_async_copy(xat_h.at[:, cols], xat.at[:, cols], sem_in.at[8 + c])

    def start_w(which, q):
        src = (wq_h, wk_h, wv_h)[which].bitcast(u32)
        for jj in range(4):
            for par in range(2):
                pltpu.make_async_copy(src.at[:, par * 16 + 4 * q + jj, :],
                                      wst.at[which * 32 + q * 8 + jj * 2 + par],
                                      sem_in.at[12 + which * 4 + q]).start()

    def cp_w(which, q):
        chunk = wst.at[pl.ds(which * 32 + q * 8, 8)]
        return pltpu.make_async_copy(chunk, chunk, sem_in.at[12 + which * 4 + q])

    def cp_wo(i):
        rows = pl.ds(pl.multiple_of(i * DM, DM), DM)
        return pltpu.make_async_copy(wot_h.at[rows, :], wot.at[rows, :], sem_in.at[24 + i])

    cp_phi.start()
    cp_wak.start()
    cp_wav.start()
    cp_xa(0).start()

    def start_batch(n):
        if n < 3:
            cp_xa(1 + n).start()
            if n == 2:
                cp_waq.start()
                cp_woa.start()
                cp_xb0.start()
                cp_mem.start()
            for q in range(4):
                start_w(n, q)
        else:
            for i in range(NP):
                cp_wo(i).start()
            cp_xb1.start()
    start_batch(0)

    pc[...] = jnp.zeros_like(pc)
    kvacc[...] = jnp.zeros_like(kvacc)
    row = _iota((DM, 640), 0)
    col = _iota((DM, 640), 1)
    perm = jnp.where(col == (row & 31) * AD + (row >> 5), 1.0, 0.0).astype(bf16)
    cp_phi.wait()
    for d in range(AD):
        pc[0:AD, 32 * d:32 * d + 32] = phi[d].astype(f32)
    rt = _dot(pc[:, 0:DM].astype(bf16), perm)
    pc[...] = rt
    rtk = pltpu.roll(rt, 64, 1)
    r2 = _iota((GR, 256), 0)
    c2 = _iota((GR, 256), 1)

    def lhead(r):
        return jnp.where(r >= 72, 4, 0) + (r & 3)

    def lidx(r):
        return jnp.where(r >= 72, r - 72, r) >> 2

    def bdt(src, g, shift):
        w = src[0:AD, 128 * g:128 * g + 256]
        w = jnp.broadcast_to(w[:, None, :], (AD, 8, 256)).reshape(9, 2, 8, 256)
        w = jnp.where(_iota((9, 8, 256), 1) < 4, w[:, 0], w[:, 1]).reshape(72, 256)
        w = jnp.concatenate([w, w], axis=0)
        rel = c2 + (128 * g - shift - GR * g) - lhead(r2) * AD
        return jnp.where((rel >= 0) & (rel < AD), w, 0.0).astype(bf16)

    bk = [bdt(rtk, g, 64) for g in range(G)]
    cp_wak.wait()
    for g in range(G):
        wk_g = _dot_nt(bk[g], _b(wa[:, 512 + 128 * g:512 + 128 * g + 256]))
        wkv[GR * g:GR * g + 72, :] = _u(wk_g.astype(bf16))
    cp_wav.wait()
    for g in range(G):
        pv = jnp.where(c2 + (128 * g - GR * g) == lhead(r2) * AD + lidx(r2), 1.0, 0.0).astype(bf16)
        kw = 256 if g < 3 else 192
        wv_g = _dot_nt(pv[:, :kw], _b(wa[:, 1152 + 128 * g:1152 + 128 * g + kw]))
        wkv[GR * g + 72:GR * g + 144, :] = _u(wv_g.astype(bf16))

    ones8 = jnp.ones((8, 512), f32)

    def relayout(which, q, piece, tok):
        jj, half = piece // 2, piece % 2
        rows = pl.ds(half * GR, GR)
        ev = wst[which * 32 + q * 8 + jj * 2, rows, :].reshape(AD, 8, E) | tok[None]
        od = wst[which * 32 + q * 8 + jj * 2 + 1, rows, :].reshape(AD, 8, E) | tok[None]
        c0 = pl.multiple_of((4 * q + jj) * 768 + which * 128, 128)
        wqkv[rows, pl.ds(c0, 128)] = ((ev & u32(0xFFFF)) | (od << 16)).reshape(GR, E)
        wqkv[rows, pl.ds(c0 + 384, 128)] = ((ev >> 16) | (od & u32(0xFFFF0000))).reshape(GR, E)

    def token(y, n):
        bits = pltpu.bitcast(y[0:8, 128 * n:128 * n + 128], u32)
        return bits & (bits + 1) & 1

    def a1_step(j, g, gprev, par, side=None):
        pk_w, pk_r = (pkb0, pkb1) if par == 0 else (pkb1, pkb0)
        va_w, va_r = (vab0, vab1) if par == 0 else (vab1, vab0)
        if g is not None:
            xt = _b(xat[:, pl.ds(pl.multiple_of(512 * j, 512), 512)])
            r0 = g * GR
            pk = _dot(_b(wkv[pl.ds(r0, 72), :]), xt)
            pk_w[...] = pk
            if side is not None:
                for n in range(4):
                    side(n, token(pk, n))
        if gprev is not None:
            ph = _features(pk_r[...])
            for g2 in range(2):
                kvacc[2 * gprev + g2] += _dot_nt(_b(va_r[g2]), ph[g2])
        if g is not None:
            v = _dot(_b(wkv[pl.ds(r0 + 72, 72), :]), xt)
            for g2 in range(2):
                va_w[g2] = _u(jnp.concatenate([v[72 * g2:72 * g2 + 72], ones8], axis=0).astype(bf16))
            if side is not None:
                for n in range(4):
                    side(4 + n, token(v, n))

    pkb1[...] = jnp.zeros_like(pkb1)
    vab1[...] = jnp.zeros_like(vab1)

    def a1_block(j, carry, rel):
        for jb in ((2, 3) if rel else (1,)):
            @pl.when(j == jb)
            def _():
                start_batch(jb)
        cp_xa(j).wait()
        if rel:
            for q in range(4):
                cp_w(j - 2, q).wait()
        for q in range(4):
            a1_step(j, q, (q + 3) % 4, q % 2, functools.partial(relayout, j - 2, q) if rel else None)
        return carry
    lax.fori_loop(0, 2, functools.partial(a1_block, rel=False), 0)
    lax.fori_loop(2, 4, functools.partial(a1_block, rel=True), 0)

    def xtrans(gidx):
        c0 = pl.multiple_of(gidx * 128, 128)
        xnat[pl.ds(c0, 128), :] = _b(xbt[:, pl.ds(c0, 128)]).astype(f32).T

    cp_waq.wait()
    cp_woa.wait()
    cp_xb0.wait()
    cp_mem.wait()
    r3 = _iota((GR, GR), 0)
    c3 = _iota((GR, GR), 1)
    pw = jnp.where(c3 == lhead(r3) * AD + lidx(r3), 1.0, 0.0).astype(bf16)
    for g in range(G):
        cp_w(2, g).wait()
        wq_g = _dot_nt(bdt(pc, g, 0), _b(wa[:, 128 * g:128 * g + 256]))
        wqt[72 * g:72 * g + 72, :] = _u(wq_g.astype(bf16))
        if g == 0:
            a1_step(None, None, 3, 0)
        wo_g = _dot(pw, _b(woa[72 * g:72 * g + 72, :]))
        wop[72 * g:72 * g + 72, :] = _u(wo_g.astype(bf16))
        for n in range(4):
            relayout(2, g, n, token(wq_g, n))
            relayout(2, g, 4 + n, token(wo_g, n))
    r4 = _iota((80, GR), 0)
    c4 = _iota((80, GR), 1)
    for g in range(2 * G):
        kvt[g] = _u(jnp.where((r4 & 3) == (c4 & 3), kvacc[g], 0.0).astype(bf16))
    xtrans(0)
    xtrans(1)
    ri = _iota((80, 80), 0)
    ci = _iota((80, 80), 1)
    same = (ri < 40) == (ci < 40)
    valid = same & (((ri >= 32) & (ri < 48)) | ((ci >= 32) & (ci < 48)) | (ci <= ri))
    fill[...] = jnp.where(valid, 0.0, jnp.where(same, -1e9 / SCALE, -jnp.inf)).astype(f32)

    def W(c0, n):
        return _b(wqkv[:, pl.ds(c0, n)])

    def WO(r0, n):
        return _b(wo32[r0 // 2:(r0 + n) // 2, :])

    def wot_rem(h):
        r0 = h * (DM // 2) + 256
        return _b(wot[pl.ds(r0 if isinstance(r0, int) else pl.multiple_of(r0, 8), 32), :])

    def tails(p):
        return jnp.concatenate(
            [xnat[pl.ds(pl.multiple_of(128 * p + 32 * c + 24, 8), 8), :] for c in range(4)], axis=0)

    lhs0 = jnp.concatenate([tails(0), xnat[0:32, :]], axis=0).astype(bf16)

    def pro(i, c):
        cp_wo(2 * i).wait()
        cp_wo(2 * i + 1).wait()
        for k in range(2):
            c0 = pl.multiple_of((2 * i + k) * 768, 128)
            y = _dot(lhs0, W(c0, 768))
            ringB[0, :, pl.ds(c0, 768)] = y[0:32]
            A0[0:24, pl.ds(c0, 768)] = y[32:56]
        for hh in range(4):
            h = 4 * i + hh
            blk = _b(wot[pl.ds(pl.multiple_of(h * (DM // 2), 8), 256), :])
            wo32[pl.ds(pl.multiple_of(h * 64, 64), 64), :] = _u(blk.T)
        for k in range(2):
            rem = jnp.concatenate([wot_rem(4 * i + 2 * k), wot_rem(4 * i + 2 * k + 1)], axis=0)
            wor[2 * i + k] = _u(rem.T)
        return c
    lax.fori_loop(0, 8, pro, 0)

    def out_copy(gidx):
        r0 = pl.multiple_of(gidx * 128, 128)
        return pltpu.make_async_copy(outb.at[pl.ds(r0, 128), :], out_h.at[pl.ds(r0, 128), :], sem_out.at[gidx])

    def period(p, mem):
        pn = jnp.minimum(p + 1, NPER - 1)
        pcur = p % 2
        pnx = 1 - pcur
        xo = tails(pn).astype(bf16)
        xt = _b(xat[:, pl.ds(pl.multiple_of(p * 128, 128), 128)])
        st = {"rt": None}

        st["ph"] = []

        def a2_pq(gs=(0, 1, 2, 3)):
            for g in gs:
                st["ph"] += _features(_dot(_b(wqt[72 * g:72 * g + 72, :]), xt))

        def a2_num():
            os_ = []
            for g in range(2 * G):
                nd = _dot(_b(kvt[g]), st["ph"][g])
                rden = 1.0 / (nd[72:80] + 1e-6)
                os_.append((nd[0:72].reshape(9, 8, 128) * rden[None]).reshape(72, 128))
            st["oa"] = jnp.concatenate(os_, axis=0).T.astype(bf16)

        def a2_out():
            y = _dot(st["oa"], _b(wop[...]))
            outb[pl.ds(pl.multiple_of(p * 128, 128), 128), 0:DM] = y.astype(bf16)

        a_stage = {0: a2_pq, 1: None, 2: a2_num, 3: a2_out}

        for r in range(4):
            Ac, An = (A0, A1) if r % 2 == 0 else (A1, A0)
            t = 4 * p + r
            tn = jnp.minimum(t + 1, 4 * NPER - 1)
            xn = xnat[pl.ds(pl.multiple_of(32 * tn, 32), 24), :]
            lhs = jnp.concatenate([mem, xn], axis=0).astype(bf16)
            fl = fill[...]
            Ac[24:32, :] = ringB[pcur, 8 * r:8 * r + 8, :]
            ys, ps, os_ = {}, {}, {}
            acc = [None, None]

            def st_qkv(i):
                y = _dot(lhs, W(768 * i, 768))
                An[0:24, 768 * i:768 * (i + 1)] = y[8:32]
                ys[i] = y[0:8]

            def gather(i, ym, o1):
                c1 = 768 * i + o1
                o2 = o1 + 384
                return jnp.concatenate([Ac[:, c1:c1 + 128], ym[:, o1:o1 + 128], ym[:, o2:o2 + 128],
                                        Ac[:, c1 + 384:c1 + 512]], axis=0).astype(bf16)

            def st_qk(i):
                s = _dot_nt(gather(i, ys[i], 0), gather(i, ys[i], 128))
                s = jnp.where(fl == 0.0, s, fl)
                m = jnp.max(s, axis=-1, keepdims=True)
                e = jnp.exp2((s - m) * (SCALE * LOG2E))
                ps[i] = (e.astype(bf16), jnp.sum(e, axis=-1, keepdims=True))

            def st_pv(i):
                e, l = ps.pop(i)
                os_[i] = _dot(e, gather(i, ys.pop(i), 256)) * (1.0 / l)

            def st_o(i):
                o = os_.pop(i)
                om, ox = (o[32:40], o[40:48]), (o[0:32], o[48:80])
                cols = [slice(256 * i + 128 * hh, 256 * i + 128 * hh + 128) for hh in range(2)]
                if r % 2 == 0:
                    lo = [jnp.concatenate([om[hh], ox[hh][0:24]], axis=0) for hh in range(2)]
                    for hh in range(2):
                        odef[:, cols[hh]] = ox[hh][24:32]
                else:
                    lo = [jnp.concatenate([om[hh], odef[:, cols[hh]], ox[hh]], axis=0) for hh in range(2)]
                y = _dot(jnp.concatenate(lo, axis=1).astype(bf16), WO(256 * i, 256))
                acc[0] = y if acc[0] is None else acc[0] + y
                y = _dot(o[32:48].astype(bf16), _b(wor[i]))
                acc[1] = y if acc[1] is None else acc[1] + y
                oxb = jnp.concatenate(ox, axis=1).astype(bf16)
                if r < 3:
                    obuf[16 * r:16 * r + 16, 256 * i:256 * i + 256] = _u(oxb)
                else:
                    blk = jnp.concatenate([_b(obuf[:, 256 * i:256 * i + 256]), oxb], axis=0)
                    y = _dot_nt(jnp.concatenate([wot_rem(2 * i), wot_rem(2 * i + 1)], axis=1), blk)
                    st["rt"] = y if st["rt"] is None else st["rt"] + y

            def f_xqkv(j):
                c0 = r * 3072 + 768 * j
                ringB[pnx, :, c0:c0 + 768] = _dot(xo, W(c0, 768))

            def f_a():
                if a_stage[r] is not None:
                    a_stage[r]()

            fn = {"0": lambda: f_xqkv(0), "1": lambda: f_xqkv(1), "2": lambda: f_xqkv(2), "3": lambda: f_xqkv(3),
                  "a": f_a}
            fillers = [[fn[c] for c in grp] for grp in "0,1,2,a3".split(",")]
            l1, l2, l3 = 1, 2, 3
            for i in range(NP + len(fillers)):
                if i < NP:
                    st_qkv(i)
                else:
                    for f in fillers[i - NP]:
                        f()
                if 0 <= i - l1 < NP:
                    st_qk(i - l1)
                if 0 <= i - l2 < NP:
                    st_pv(i - l2)
                if 0 <= i - l3 < NP:
                    st_o(i - l3)
            assert not os_ and not ps and not ys
            if r % 2 == 0:
                outb[pl.ds(pl.multiple_of(32 * t, 32), 24), DM:DM + 512] = acc[0][8:32].astype(bf16)
            else:
                outb[pl.ds(pl.multiple_of(32 * t - 8, 8), 40), DM:DM + 512] = acc[0][8:48].astype(bf16)
            mrem = acc[1][0:8] + pltpu.roll(acc[1][8:16], 64, 1)
            mem = jnp.concatenate([acc[0][0:8], mrem[:, 0:64]], axis=1)

        rt = jnp.concatenate([jnp.zeros((64, 128), f32), st["rt"]], axis=0).T
        outb[pl.ds(pl.multiple_of(p * 128, 128), 128), DM + 512:2 * DM] = rt[:, 64:128].astype(bf16)
        xtrans(jnp.minimum(p + 2, NPER - 1))
        out_copy(p).start()

        @pl.when(p == 0)
        def _():
            cp_xb1.wait()
        return mem

    lax.fori_loop(0, nper, period, mem0[...].astype(f32))
    for gidx in range(nper):
        out_copy(gidx).wait()


def build(nper=NPER):
    V = pltpu.VMEM
    scratch = [
        V((DM // 2, S), u32),
        V((DM // 2, 3 * DM), u32),
        V((AD, AD, AH), bf16),
        V((DM // 2, DM), u32),
        V((DM // 2, S), u32),
        V((M, DM), bf16),
        V((3 * H, DM // 2, E), u32),
        V((H * DM // 2, E), u32),
        V((32, 640), f32),
        V((DM, DM), u32),
        V((DM // 2, DM), u32),
        V((DM // 2, DM), u32),
        V((2 * G, 80, GR), f32),
        V((2 * G, 40, GR), u32),
        V((GR, 512), f32),
        V((GR, 512), f32),
        V((2, 40, 512), u32),
        V((2, 40, 512), u32),
        V((DM // 2, 3 * H * E), u32),
        V((H * E // 2, 512), u32),
        V((NP, 64, E), u32),
        V((S, DM), f32),
        V((32, 3 * H * E), f32),
        V((32, 3 * H * E), f32),
        V((2, 32, 3 * H * E), f32),
        V((8, H * E), f32),
        V((48, H * E), u32),
        V((80, 80), f32),
        V((S, 2 * DM), bf16),
        pltpu.SemaphoreType.DMA((8 + 4 + 12 + NP,)),
        pltpu.SemaphoreType.DMA((NPER,)),
    ]

    def fn(A_x, A_wqkv, A_w_phi, A_wo, B_x, B_mem0, B_Wq, B_Wk, B_Wv, B_Wo):
        out = pl.pallas_call(
            functools.partial(_kernel, nper=nper),
            out_shape=jax.ShapeDtypeStruct((S, 2 * DM), bf16),
            in_specs=[pl.BlockSpec(memory_space=pl.ANY)] * 10,
            out_specs=pl.BlockSpec(memory_space=pl.ANY),
            scratch_shapes=scratch,
            compiler_params=pltpu.CompilerParams(vmem_limit_bytes=112 * 1024 * 1024),
        )(
            jnp.swapaxes(A_x, 1, 2).reshape(DM, S),
            A_wqkv,
            jnp.transpose(A_w_phi, (1, 2, 0)),
            A_wo,
            jnp.swapaxes(B_x, 1, 2).reshape(DM, S),
            B_mem0.reshape(M, DM),
            B_Wq.reshape(DM // 2, 2 * H, E),
            B_Wk.reshape(DM // 2, 2 * H, E),
            B_Wv.reshape(DM // 2, 2 * H, E),
            jnp.swapaxes(B_Wo, 1, 2).reshape(H * DM, E),
        )
        return out.reshape(1, S, 2 * DM)
    return fn


@functools.partial(jax.jit, static_argnames=("B_seg_len",))
def pallas_concat_heads__linear_kernel_hedgehog__memory_aug_recurrent_mem_tr__prompt_kernel(
    A_x, A_wqkv, A_w_phi, A_wo, B_x, B_mem0, B_Wq, B_Wk, B_Wv, B_Wo, B_seg_len,
):
    assert B_seg_len == SEG and A_x.shape == (1, S, DM) and B_x.shape == (1, S, DM)
    return build()(A_x, A_wqkv, A_w_phi, A_wo, B_x, B_mem0, B_Wq, B_Wk, B_Wv, B_Wo)
```

```python
import functools
import jax
import jax.numpy as jnp
from jax import lax
from jax.experimental import pallas as pl
from jax.experimental.pallas import tpu as pltpu

f32, bf16, u32, i32 = jnp.float32, jnp.bfloat16, jnp.uint32, jnp.int32

S, DM = 2048, 576
H, E, M, SEG = 32, 128, 8, 32
NP = H // 2
NPER = S // (4 * SEG)
AH, AD = 32, 18
G, GR = 4, 144
NE = 1
PU = 2
NT = 2
SCALE = float(E) ** -0.5
LOG2E = 1.4426950408889634


def _dot(a, b):
    return jnp.dot(a, b, preferred_element_type=f32)


def _dot_nt(a, b):
    return lax.dot_general(a, b, (((1,), (1,)), ((), ())), preferred_element_type=f32)


def _b(x):
    return pltpu.bitcast(x, bf16)


def _u(x):
    return pltpu.bitcast(x, u32)


def _iota(shape, dim):
    return lax.broadcasted_iota(i32, shape, dim)


def _features(p):
    t = p.shape[1]
    outs = []
    for g2 in range(2):
        x3 = p[72 * g2:72 * g2 + 72].reshape(9, 8, t)
        mx = jnp.max(x3, axis=0)
        mx = jnp.maximum(mx, pltpu.roll(mx, 4, 0))
        mn = jnp.min(x3, axis=0)
        mn = jnp.minimum(mn, pltpu.roll(mn, 4, 0))
        ep = jnp.exp(x3 - mx[None])
        en = jnp.exp(mn[None] - x3)
        sp = jnp.sum(ep, axis=0)
        sn = jnp.sum(en, axis=0)
        rp = 1.0 / (sp + pltpu.roll(sp, 4, 0))
        rn = 1.0 / (sn + pltpu.roll(sn, 4, 0))
        phi = jnp.concatenate([ep * rp[None], en * rn[None]], axis=0)
        outs.append(phi.reshape(GR, t).astype(bf16))
    return outs


def _kernel(xat_h, wa_h, phi_h, woa_h, xbt_h, mem_h, wq_h, wk_h, wv_h, wot_h, out_h,
            xat, wa, phi, woa, xbt, mem0, wst, wot,
            pc, wkv, wqt, wop, wopt, kvacc, kvt, pqb, pkb0, pkb1, vab0, vab1,
            wqkv, wo32, wor, xnat, A0, A1, ringB, odef, obuf, fill, outb,
            sem_in, sem_out, *, nper):
    xat_h, wa_h, woa_h, xbt_h, wot_h = [r.bitcast(u32) for r in (xat_h, wa_h, woa_h, xbt_h, wot_h)]
    cp_phi = pltpu.make_async_copy(phi_h, phi, sem_in.at[0])
    cp_wak = pltpu.make_async_copy(wa_h.at[:, 512:1152], wa.at[:, 512:1152], sem_in.at[1])
    cp_wav = pltpu.make_async_copy(wa_h.at[:, 1152:1728], wa.at[:, 1152:1728], sem_in.at[2])
    cp_waq = pltpu.make_async_copy(wa_h.at[:, 0:512], wa.at[:, 0:512], sem_in.at[3])
    cp_woa = pltpu.make_async_copy(woa_h, woa, sem_in.at[4])
    cp_mem = pltpu.make_async_copy(mem_h, mem0, sem_in.at[5])
    cp_xb0 = pltpu.make_async_copy(xbt_h.at[:, 0:384], xbt.at[:, 0:384], sem_in.at[6])
    cp_xb1 = pltpu.make_async_copy(xbt_h.at[:, 384:S], xbt.at[:, 384:S], sem_in.at[7])

    def cp_xa(c):
        cols = pl.ds(pl.multiple_of(c * 512, 512), 512)
        return pltpu.make_async_copy(xat_h.at[:, cols], xat.at[:, cols], sem_in.at[8 + c])

    def start_w(which, q):
        src = (wq_h, wk_h, wv_h)[which].bitcast(u32)
        for jj in range(4):
            for par in range(2):
                pltpu.make_async_copy(src.at[:, par * 16 + 4 * q + jj, :],
                                      wst.at[which * 32 + q * 8 + jj * 2 + par],
                                      sem_in.at[12 + which * 4 + q]).start()

    def cp_w(which, q):
        chunk = wst.at[pl.ds(which * 32 + q * 8, 8)]
        return pltpu.make_async_copy(chunk, chunk, sem_in.at[12 + which * 4 + q])

    def cp_wo(i):
        rows = pl.ds(pl.multiple_of(i * DM, DM), DM)
        return pltpu.make_async_copy(wot_h.at[rows, :], wot.at[rows, :], sem_in.at[24 + i])

    cp_phi.start()
    cp_wak.start()
    cp_wav.start()
    cp_xa(0).start()

    def start_batch(n):
        if n < 3:
            cp_xa(1 + n).start()
            if n == 2:
                cp_waq.start()
                cp_woa.start()
                cp_xb0.start()
                cp_mem.start()
            for q in range(4):
                start_w(n, q)
        else:
            for i in range(NP):
                cp_wo(i).start()
            cp_xb1.start()
    start_batch(0)

    pc[...] = jnp.zeros_like(pc)
    kvacc[...] = jnp.zeros_like(kvacc)
    row = _iota((DM, 640), 0)
    col = _iota((DM, 640), 1)
    perm = jnp.where(col == (row & 31) * AD + (row >> 5), 1.0, 0.0).astype(bf16)
    cp_phi.wait()
    for d in range(AD):
        pc[0:AD, 32 * d:32 * d + 32] = phi[d].astype(f32)
    rt = _dot(pc[:, 0:DM].astype(bf16), perm)
    pc[...] = rt
    rtk = pltpu.roll(rt, 64, 1)

    def window(hg, shift):
        lo = shift + 72 * hg
        c0 = lo // 128 * 128
        return c0, min((lo + 71) // 128 * 128 + 128, shift + DM) - c0

    def fold(hg, shift, base, src):
        c0, n = window(hg, shift)
        r2 = _iota((72, n), 0)
        rel = _iota((72, n), 1) + (c0 - shift - 72 * hg) - (r2 & 3) * AD
        if src is None:
            sel = jnp.where(rel == (r2 >> 2), 1.0, 0.0)
        else:
            w = jnp.broadcast_to(src[0:AD, c0:c0 + n][:, None, :], (AD, 8, n)).reshape(9, 2, 8, n)
            w = jnp.where(_iota((9, 8, n), 1) < 4, w[:, 0], w[:, 1]).reshape(72, n)
            sel = jnp.where((rel >= 0) & (rel < AD), w, 0.0)
        return _dot_nt(sel.astype(bf16), _b(wa[:, base + c0:base + c0 + n]))

    def fold2(g, shift, base, src):
        return jnp.concatenate([fold(2 * g, shift, base, src), fold(2 * g + 1, shift, base, src)], axis=0)

    cp_wak.wait()
    for g in range(G):
        wkv[GR * g:GR * g + 72, :] = _u(fold2(g, 64, 512, rtk).astype(bf16))
    cp_wav.wait()
    for g in range(G):
        wkv[GR * g + 72:GR * g + 144, :] = _u(fold2(g, 0, 1152, None).astype(bf16))

    ones8 = jnp.ones((8, 512), f32)

    def relayout(which, q, piece, tok):
        jj, half = piece // 2, piece % 2
        c0 = pl.multiple_of((4 * q + jj) * 768 + which * 128, 128)
        for k in range(NT):
            n = GR // NT
            rows = pl.ds(half * GR + k * n, n)
            ev = wst[which * 32 + q * 8 + jj * 2, rows, :].reshape(n // 8, 8, E) | tok[k][None]
            od = wst[which * 32 + q * 8 + jj * 2 + 1, rows, :].reshape(n // 8, 8, E) | tok[k][None]
            wqkv[rows, pl.ds(c0, 128)] = ((ev & u32(0xFFFF)) | (od << 16)).reshape(n, E)
            wqkv[rows, pl.ds(c0 + 384, 128)] = ((ev >> 16) | (od & u32(0xFFFF0000))).reshape(n, E)

    def token(y, n):
        out = []
        for k in range(NT):
            r = (GR // NT) * k
            bits = pltpu.bitcast(y[r:r + 8, 128 * n:128 * n + 128], u32)
            out.append(bits & (bits + 1) & 1)
        return out

    def a1_step(j, g, gprev, par, side=None):
        pk_w, pk_r = (pkb0, pkb1) if par == 0 else (pkb1, pkb0)
        va_w, va_r = (vab0, vab1) if par == 0 else (vab1, vab0)
        if g is not None:
            xt = _b(xat[:, pl.ds(pl.multiple_of(512 * j, 512), 512)])
            r0 = g * GR
            pk = _dot(_b(wkv[pl.ds(r0, 72), :]), xt)
            pk_w[...] = pk
            if side is not None:
                for n in range(4):
                    side(n, token(pk, n))
        if gprev is not None:
            ph = _features(pk_r[...])
            for g2 in range(2):
                kvacc[2 * gprev + g2] += _dot_nt(_b(va_r[g2]), ph[g2])
        if g is not None:
            v = _dot(_b(wkv[pl.ds(r0 + 72, 72), :]), xt)
            for g2 in range(2):
                va_w[g2] = _u(jnp.concatenate([v[72 * g2:72 * g2 + 72], ones8], axis=0).astype(bf16))
            if side is not None:
                for n in range(4):
                    side(4 + n, token(v, n))

    pkb1[...] = jnp.zeros_like(pkb1)
    vab1[...] = jnp.zeros_like(vab1)

    def a1_block(j, carry, rel):
        for jb in ((2, 3) if rel else (1,)):
            @pl.when(j == jb)
            def _():
                start_batch(jb)
        cp_xa(j).wait()
        if rel:
            for q in range(4):
                cp_w(j - 2, q).wait()
        for q in range(4):
            a1_step(j, q, (q + 3) % 4, q % 2, functools.partial(relayout, j - 2, q) if rel else None)
        return carry
    lax.fori_loop(0, 2, functools.partial(a1_block, rel=False), 0)
    lax.fori_loop(2, 4, functools.partial(a1_block, rel=True), 0)

    def xtrans(gidx):
        c0 = pl.multiple_of(gidx * 128, 128)
        xnat[pl.ds(c0, 128), :] = _b(xbt[:, pl.ds(c0, 128)]).astype(f32).T

    cp_waq.wait()
    cp_woa.wait()
    cp_xb0.wait()
    cp_mem.wait()
    r3 = _iota((72, 80), 0)
    c3 = _iota((72, 80), 1)
    pw = [jnp.where(c3 - 8 * g2 == (r3 & 3) * AD + (r3 >> 2), 1.0, 0.0).astype(bf16) for g2 in range(2)]
    def prep_wo(g):
        y = jnp.concatenate(
            [_dot(pw[g2], _b(woa[72 * g + 32 * g2:72 * g + 32 * g2 + 40, :])) for g2 in range(2)], axis=0)
        wop[72 * g:72 * g + 72, :] = _u(y.astype(bf16))
        return y

    def prep_q(g):
        y = fold2(g, 0, 0, pc)
        wqt[72 * g:72 * g + 72, :] = _u(y.astype(bf16))
        return y

    def pq_early(g, j):
        y = _dot(_b(wqt[72 * g:72 * g + 72, :]), _b(xat[:, 512 * j:512 * j + 512]))
        pqb[GR * g:GR * g + GR, 512 * j:512 * j + 512] = y
        return y

    def wo_trans(n):
        w = min(128, DM - 128 * n)
        wopt[64 * n:64 * n + w // 2, :] = _u(_b(wop[:, 128 * n:128 * n + w]).T)

    for qs, jobs in (((0, 1), [("w", g) for g in range(G)] + [("q", g) for g in range(NE)]
                      + [("e", (g, j)) for g in range(NE) for j in range(4)]),
                     ((2, 3), [("q", g) for g in range(NE, G)])):
        for q in qs:
            cp_w(2, q).wait()
        toks = []
        for k, (kind, arg) in enumerate(jobs):
            y = prep_wo(arg) if kind == "w" else prep_q(arg) if kind == "q" else pq_early(*arg)
            toks += [token(y, n) for n in range(4)]
            if qs[0] == 0 and k == 1:
                a1_step(None, None, 3, 0)
        for n in range(16):
            relayout(2, qs[n // 8], n % 8, toks[n * len(toks) // 16])
        for n in ((0, 1, 2) if qs[0] == 0 else (3, 4)):
            wo_trans(n)
    r4 = _iota((80, GR), 0)
    c4 = _iota((80, GR), 1)
    for g in range(2 * G):
        kvt[g] = _u(jnp.where((r4 & 3) == (c4 & 3), kvacc[g], 0.0).astype(bf16))
    xtrans(0)
    xtrans(1)
    ri = _iota((80, 80), 0)
    ci = _iota((80, 80), 1)
    same = (ri < 40) == (ci < 40)
    valid = same & (((ri >= 32) & (ri < 48)) | ((ci >= 32) & (ci < 48)) | (ci <= ri))
    fill[...] = jnp.where(valid, 0.0, jnp.where(same, -1e9 / SCALE, -jnp.inf)).astype(f32)

    def W(c0, n):
        return _b(wqkv[:, pl.ds(c0, n)])

    def WO(r0, n):
        return _b(wo32[r0 // 2:(r0 + n) // 2, :])

    def wot_rem(h):
        r0 = h * (DM // 2) + 256
        return _b(wot[pl.ds(r0 if isinstance(r0, int) else pl.multiple_of(r0, 8), 32), :])

    def tails(p):
        return jnp.concatenate(
            [xnat[pl.ds(pl.multiple_of(128 * p + 32 * c + 24, 8), 8), :] for c in range(4)], axis=0)

    lhs0 = jnp.concatenate([tails(0), xnat[0:32, :]], axis=0).astype(bf16)

    def pro(i, c):
        for k in range(PU):
            cp_wo(PU * i + k).wait()
        for k in range(PU):
            c0 = pl.multiple_of((PU * i + k) * 768, 128)
            y = _dot(lhs0, W(c0, 768))
            ringB[0, :, pl.ds(c0, 768)] = y[0:32]
            A0[0:24, pl.ds(c0, 768)] = y[32:56]
            for hh in range(2):
                h = 2 * (PU * i + k) + hh
                blk = _b(wot[pl.ds(pl.multiple_of(h * (DM // 2), 8), 256), :])
                wo32[pl.ds(pl.multiple_of(h * 64, 64), 64), :] = _u(blk.T)
            rem = jnp.concatenate([wot_rem(2 * (PU * i + k)), wot_rem(2 * (PU * i + k) + 1)], axis=0)
            wor[PU * i + k] = _u(rem.T)
        return c
    lax.fori_loop(0, NP // PU, pro, 0)

    def out_copy(gidx):
        r0 = pl.multiple_of(gidx * 128, 128)
        return pltpu.make_async_copy(outb.at[pl.ds(r0, 128), :], out_h.at[pl.ds(r0, 128), :], sem_out.at[gidx])

    def period(p, mem):
        pn = jnp.minimum(p + 1, NPER - 1)
        pcur = p % 2
        pnx = 1 - pcur
        xo = tails(pn).astype(bf16)
        xt = _b(xat[:, pl.ds(pl.multiple_of(p * 128, 128), 128)])
        st = {"rt": None}

        st["ph"] = {}

        def a2_pq(gs):
            for g in gs:
                if g < NE:
                    st["ph"][g] = _features(pqb[GR * g:GR * g + GR, pl.ds(pl.multiple_of(p * 128, 128), 128)])
                else:
                    st["ph"][g] = _features(_dot(_b(wqt[72 * g:72 * g + 72, :]), xt))

        def a2_num():
            os_ = []
            for g in range(2 * G):
                nd = _dot(_b(kvt[g]), st["ph"][g // 2][g % 2])
                rden = 1.0 / (nd[72:80] + 1e-6)
                os_.append((nd[0:72].reshape(9, 8, 128) * rden[None]).reshape(72, 128))
            st["oa"] = jnp.concatenate(os_, axis=0).astype(bf16)

        def a2_out():
            y = jnp.concatenate([_dot(_b(wopt[72 * g:72 * g + 72, :]), st["oa"]) for g in range(G)], axis=0)
            outb[pl.ds(pl.multiple_of(p * 128, 128), 128), 0:DM] = y.T.astype(bf16)

        a_stage = (lambda: a2_pq((0, 1)), lambda: a2_pq((2, 3)), a2_num, a2_out)

        for r in range(4):
            Ac, An = (A0, A1) if r % 2 == 0 else (A1, A0)
            t = 4 * p + r
            tn = jnp.minimum(t + 1, 4 * NPER - 1)
            xn = xnat[pl.ds(pl.multiple_of(32 * tn, 32), 24), :]
            lhs = jnp.concatenate([mem, xn], axis=0).astype(bf16)
            fl = fill[...]
            Ac[24:32, :] = ringB[pcur, 8 * r:8 * r + 8, :]
            ys, ps, os_ = {}, {}, {}
            acc = [None, None]

            def st_qkv(i):
                y = _dot(lhs, W(768 * i, 768))
                An[0:24, 768 * i:768 * (i + 1)] = y[8:32]
                ys[i] = y[0:8]

            def gather(i, ym, o1):
                c1 = 768 * i + o1
                o2 = o1 + 384
                return jnp.concatenate([Ac[:, c1:c1 + 128], ym[:, o1:o1 + 128], ym[:, o2:o2 + 128],
                                        Ac[:, c1 + 384:c1 + 512]], axis=0).astype(bf16)

            def st_qk(i):
                s = _dot_nt(gather(i, ys[i], 0), gather(i, ys[i], 128))
                s = jnp.where(fl == 0.0, s, fl)
                m = jnp.max(s, axis=-1, keepdims=True)
                e = jnp.exp2((s - m) * (SCALE * LOG2E))
                ps[i] = (e.astype(bf16), jnp.sum(e, axis=-1, keepdims=True))

            def st_pv(i):
                e, l = ps.pop(i)
                os_[i] = _dot(e, gather(i, ys.pop(i), 256)) * (1.0 / l)

            def st_o(i):
                o = os_.pop(i)
                om, ox = (o[32:40], o[40:48]), (o[0:32], o[48:80])
                cols = [slice(256 * i + 128 * hh, 256 * i + 128 * hh + 128) for hh in range(2)]
                if r % 2 == 0:
                    lo = [jnp.concatenate([om[hh], ox[hh][0:24]], axis=0) for hh in range(2)]
                    for hh in range(2):
                        odef[:, cols[hh]] = ox[hh][24:32]
                else:
                    lo = [jnp.concatenate([om[hh], odef[:, cols[hh]], ox[hh]], axis=0) for hh in range(2)]
                y = _dot(jnp.concatenate(lo, axis=1).astype(bf16), WO(256 * i, 256))
                acc[0] = y if acc[0] is None else acc[0] + y
                y = _dot(o[32:48].astype(bf16), _b(wor[i]))
                acc[1] = y if acc[1] is None else acc[1] + y
                oxb = jnp.concatenate(ox, axis=1).astype(bf16)
                if r < 3:
                    obuf[16 * r:16 * r + 16, 256 * i:256 * i + 256] = _u(oxb)
                else:
                    blk = jnp.concatenate([_b(obuf[:, 256 * i:256 * i + 256]), oxb], axis=0)
                    y = _dot_nt(jnp.concatenate([wot_rem(2 * i), wot_rem(2 * i + 1)], axis=1), blk)
                    st["rt"] = y if st["rt"] is None else st["rt"] + y

            def f_xqkv(j):
                c0 = r * 3072 + 768 * j
                ringB[pnx, :, c0:c0 + 768] = _dot(xo, W(c0, 768))

            for i in range(NP + 4):
                if i < NP:
                    st_qkv(i)
                else:
                    if r < 3 and i == NP + 3:
                        a_stage[r]()
                    f_xqkv(i - NP)
                    if r == 3 and i == NP + 1:
                        a_stage[r]()
                if 0 <= i - 1 < NP:
                    st_qk(i - 1)
                if 0 <= i - 2 < NP:
                    st_pv(i - 2)
                if 0 <= i - 3 < NP:
                    st_o(i - 3)
            assert not os_ and not ps and not ys
            if r % 2 == 0:
                outb[pl.ds(pl.multiple_of(32 * t, 32), 24), DM:DM + 512] = acc[0][8:32].astype(bf16)
            else:
                outb[pl.ds(pl.multiple_of(32 * t - 8, 8), 40), DM:DM + 512] = acc[0][8:48].astype(bf16)
            mrem = acc[1][0:8] + pltpu.roll(acc[1][8:16], 64, 1)
            mem = jnp.concatenate([acc[0][0:8], mrem[:, 0:64]], axis=1)

        rt = jnp.concatenate([jnp.zeros((64, 128), f32), st["rt"]], axis=0).T
        outb[pl.ds(pl.multiple_of(p * 128, 128), 128), DM + 512:2 * DM] = rt[:, 64:128].astype(bf16)
        xtrans(jnp.minimum(p + 2, NPER - 1))
        out_copy(p).start()

        @pl.when(p == 0)
        def _():
            cp_xb1.wait()
        return mem

    lax.fori_loop(0, nper, period, mem0[...].astype(f32))
    for gidx in range(nper):
        out_copy(gidx).wait()


def build(nper=NPER):
    V = pltpu.VMEM
    scratch = [
        V((DM // 2, S), u32),
        V((DM // 2, 3 * DM), u32),
        V((AD, AD, AH), bf16),
        V((DM // 2, DM), u32),
        V((DM // 2, S), u32),
        V((M, DM), bf16),
        V((3 * H, DM // 2, E), u32),
        V((H * DM // 2, E), u32),
        V((32, 640), f32),
        V((DM, DM), u32),
        V((DM // 2, DM), u32),
        V((DM // 2, DM), u32),
        V((DM // 2, DM), u32),
        V((2 * G, 80, GR), f32),
        V((2 * G, 40, GR), u32),
        V((NE * GR, S), f32),
        V((GR, 512), f32),
        V((GR, 512), f32),
        V((2, 40, 512), u32),
        V((2, 40, 512), u32),
        V((DM // 2, 3 * H * E), u32),
        V((H * E // 2, 512), u32),
        V((NP, 64, E), u32),
        V((S, DM), f32),
        V((32, 3 * H * E), f32),
        V((32, 3 * H * E), f32),
        V((2, 32, 3 * H * E), f32),
        V((8, H * E), f32),
        V((48, H * E), u32),
        V((80, 80), f32),
        V((S, 2 * DM), bf16),
        pltpu.SemaphoreType.DMA((8 + 4 + 12 + NP,)),
        pltpu.SemaphoreType.DMA((NPER,)),
    ]

    def fn(A_x, A_wqkv, A_w_phi, A_wo, B_x, B_mem0, B_Wq, B_Wk, B_Wv, B_Wo):
        out = pl.pallas_call(
            functools.partial(_kernel, nper=nper),
            out_shape=jax.ShapeDtypeStruct((S, 2 * DM), bf16),
            in_specs=[pl.BlockSpec(memory_space=pl.ANY)] * 10,
            out_specs=pl.BlockSpec(memory_space=pl.ANY),
            scratch_shapes=scratch,
            compiler_params=pltpu.CompilerParams(vmem_limit_bytes=112 * 1024 * 1024),
        )(
            jnp.swapaxes(A_x, 1, 2).reshape(DM, S),
            A_wqkv,
            jnp.transpose(A_w_phi, (1, 2, 0)),
            A_wo,
            jnp.swapaxes(B_x, 1, 2).reshape(DM, S),
            B_mem0.reshape(M, DM),
            B_Wq.reshape(DM // 2, 2 * H, E),
            B_Wk.reshape(DM // 2, 2 * H, E),
            B_Wv.reshape(DM // 2, 2 * H, E),
            jnp.swapaxes(B_Wo, 1, 2).reshape(H * DM, E),
        )
        return out.reshape(1, S, 2 * DM)
    return fn


_impl = jax.jit(build())


def pallas_concat_heads__linear_kernel_hedgehog__memory_aug_recurrent_mem_tr__prompt_kernel(
    A_x, A_wqkv, A_w_phi, A_wo, B_x, B_mem0, B_Wq, B_Wk, B_Wv, B_Wo, B_seg_len,
):
    if isinstance(B_seg_len, int):
        assert B_seg_len == SEG
    assert A_x.shape == (1, S, DM) and B_x.shape == (1, S, DM) and B_mem0.shape == (1, M, DM)
    return _impl(A_x, A_wqkv, A_w_phi, A_wo, B_x, B_mem0, B_Wq, B_Wk, B_Wv, B_Wo)
```

```python
import functools
import jax
import jax.numpy as jnp
from jax import lax
from jax.experimental import pallas as pl
from jax.experimental.pallas import tpu as pltpu

f32, bf16, u32, i32 = jnp.float32, jnp.bfloat16, jnp.uint32, jnp.int32

S, DM = 2048, 576
H, E, M, SEG = 32, 128, 8, 32
NP = H // 2
NPER = S // (4 * SEG)
AH, AD = 32, 18
G, GR = 4, 144
NE = 1
PU = 2
NT = 2
SCALE = float(E) ** -0.5
LOG2E = 1.4426950408889634


def _dot(a, b):
    return jnp.dot(a, b, preferred_element_type=f32)


def _dot_nt(a, b):
    return lax.dot_general(a, b, (((1,), (1,)), ((), ())), preferred_element_type=f32)


def _b(x):
    return pltpu.bitcast(x, bf16)


def _u(x):
    return pltpu.bitcast(x, u32)


def _iota(shape, dim):
    return lax.broadcasted_iota(i32, shape, dim)


def _features(p):
    t = p.shape[1]
    outs = []
    for g2 in range(2):
        x3 = p[72 * g2:72 * g2 + 72].reshape(9, 8, t)
        mx = jnp.max(x3, axis=0)
        mx = jnp.maximum(mx, pltpu.roll(mx, 4, 0))
        mn = jnp.min(x3, axis=0)
        mn = jnp.minimum(mn, pltpu.roll(mn, 4, 0))
        ep = jnp.exp(x3 - mx[None])
        en = jnp.exp(mn[None] - x3)
        sp = jnp.sum(ep, axis=0)
        sn = jnp.sum(en, axis=0)
        rp = 1.0 / (sp + pltpu.roll(sp, 4, 0))
        rn = 1.0 / (sn + pltpu.roll(sn, 4, 0))
        phi = jnp.concatenate([ep * rp[None], en * rn[None]], axis=0)
        outs.append(phi.reshape(GR, t).astype(bf16))
    return outs


def _kernel(xat_h, wa_h, phi_h, woa_h, xbt_h, mem_h, wq_h, wk_h, wv_h, wot_h, out_h,
            xat, wa, phi, woa, xbt, mem0, wst, wot,
            pc, wkv, wqt, wop, wopt, kvacc, kvt, pqb, pkb0, pkb1, vab0, vab1,
            wqkv, wo32, wor, xnat, A0, A1, ringB, odef, obuf, fill, outb,
            sem_in, sem_out, *, nper):
    xat_h, wa_h, woa_h, xbt_h, wot_h = [r.bitcast(u32) for r in (xat_h, wa_h, woa_h, xbt_h, wot_h)]
    cp_phi = pltpu.make_async_copy(phi_h, phi, sem_in.at[0])
    cp_wak = pltpu.make_async_copy(wa_h.at[:, 512:1152], wa.at[:, 512:1152], sem_in.at[1])
    cp_wav = pltpu.make_async_copy(wa_h.at[:, 1152:1728], wa.at[:, 1152:1728], sem_in.at[2])
    cp_waq = pltpu.make_async_copy(wa_h.at[:, 0:512], wa.at[:, 0:512], sem_in.at[3])
    cp_woa = pltpu.make_async_copy(woa_h, woa, sem_in.at[4])
    cp_mem = pltpu.make_async_copy(mem_h, mem0, sem_in.at[5])
    cp_xb0 = pltpu.make_async_copy(xbt_h.at[:, 0:384], xbt.at[:, 0:384], sem_in.at[6])
    cp_xb1 = pltpu.make_async_copy(xbt_h.at[:, 384:S], xbt.at[:, 384:S], sem_in.at[7])

    def cp_xa(c):
        cols = pl.ds(pl.multiple_of(c * 512, 512), 512)
        return pltpu.make_async_copy(xat_h.at[:, cols], xat.at[:, cols], sem_in.at[8 + c])

    def start_w(which, q):
        src = (wq_h, wk_h, wv_h)[which].bitcast(u32)
        for jj in range(4):
            for par in range(2):
                pltpu.make_async_copy(src.at[:, par * 16 + 4 * q + jj, :],
                                      wst.at[which * 32 + q * 8 + jj * 2 + par],
                                      sem_in.at[12 + which * 4 + q]).start()

    def cp_w(which, q):
        chunk = wst.at[pl.ds(which * 32 + q * 8, 8)]
        return pltpu.make_async_copy(chunk, chunk, sem_in.at[12 + which * 4 + q])

    def cp_wo(i):
        rows = pl.ds(pl.multiple_of(i * DM, DM), DM)
        return pltpu.make_async_copy(wot_h.at[rows, :], wot.at[rows, :], sem_in.at[24 + i])

    cp_phi.start()
    cp_wak.start()
    cp_wav.start()
    cp_xa(0).start()

    def start_batch(n):
        if n < 3:
            cp_xa(1 + n).start()
            if n == 2:
                cp_waq.start()
                cp_woa.start()
                cp_xb0.start()
                cp_mem.start()
            for q in range(4):
                start_w(n, q)
        else:
            for i in range(NP):
                cp_wo(i).start()
            cp_xb1.start()
    start_batch(0)

    pc[...] = jnp.zeros_like(pc)
    kvacc[...] = jnp.zeros_like(kvacc)
    row = _iota((DM, 640), 0)
    col = _iota((DM, 640), 1)
    perm = jnp.where(col == (row & 31) * AD + (row >> 5), 1.0, 0.0).astype(bf16)
    cp_phi.wait()
    for d in range(AD):
        pc[0:AD, 32 * d:32 * d + 32] = phi[d].astype(f32)
    rt = _dot(pc[:, 0:DM].astype(bf16), perm)
    pc[...] = rt
    rtk = pltpu.roll(rt, 64, 1)

    def window(hg, shift):
        lo = shift + 72 * hg
        c0 = lo // 128 * 128
        return c0, min((lo + 71) // 128 * 128 + 128, shift + DM) - c0

    def fold(hg, shift, base, src):
        c0, n = window(hg, shift)
        r2 = _iota((72, n), 0)
        rel = _iota((72, n), 1) + (c0 - shift - 72 * hg) - (r2 & 3) * AD
        if src is None:
            sel = jnp.where(rel == (r2 >> 2), 1.0, 0.0)
        else:
            w = jnp.broadcast_to(src[0:AD, c0:c0 + n][:, None, :], (AD, 8, n)).reshape(9, 2, 8, n)
            w = jnp.where(_iota((9, 8, n), 1) < 4, w[:, 0], w[:, 1]).reshape(72, n)
            sel = jnp.where((rel >= 0) & (rel < AD), w, 0.0)
        return _dot_nt(sel.astype(bf16), _b(wa[:, base + c0:base + c0 + n]))

    def fold2(g, shift, base, src):
        return jnp.concatenate([fold(2 * g, shift, base, src), fold(2 * g + 1, shift, base, src)], axis=0)

    cp_wak.wait()
    for g in range(G):
        wkv[GR * g:GR * g + 72, :] = _u(fold2(g, 64, 512, rtk).astype(bf16))
    cp_wav.wait()
    for g in range(G):
        wkv[GR * g + 72:GR * g + 144, :] = _u(fold2(g, 0, 1152, None).astype(bf16))

    ones8 = jnp.ones((8, 512), f32)

    def relayout(which, q, piece, tok):
        jj, half = piece // 2, piece % 2
        c0 = pl.multiple_of((4 * q + jj) * 768 + which * 128, 128)
        for k in range(NT):
            n = GR // NT
            rows = pl.ds(half * GR + k * n, n)
            ev = wst[which * 32 + q * 8 + jj * 2, rows, :].reshape(n // 8, 8, E) | tok[k][None]
            od = wst[which * 32 + q * 8 + jj * 2 + 1, rows, :].reshape(n // 8, 8, E) | tok[k][None]
            wqkv[rows, pl.ds(c0, 128)] = ((ev & u32(0xFFFF)) | (od << 16)).reshape(n, E)
            wqkv[rows, pl.ds(c0 + 384, 128)] = ((ev >> 16) | (od & u32(0xFFFF0000))).reshape(n, E)

    def token(y, n):
        out = []
        for k in range(NT):
            r = (GR // NT) * k
            bits = pltpu.bitcast(y[r:r + 8, 128 * n:128 * n + 128], u32)
            out.append(bits & (bits + 1) & 1)
        return out

    def a1_step(j, g, gprev, par, side=None):
        pk_w, pk_r = (pkb0, pkb1) if par == 0 else (pkb1, pkb0)
        va_w, va_r = (vab0, vab1) if par == 0 else (vab1, vab0)
        if g is not None:
            xt = _b(xat[:, pl.ds(pl.multiple_of(512 * j, 512), 512)])
            r0 = g * GR
            pk = _dot(_b(wkv[pl.ds(r0, 72), :]), xt)
            pk_w[...] = pk
            if side is not None:
                for n in range(4):
                    side(n, token(pk, n))
        if gprev is not None:
            ph = _features(pk_r[...])
            for g2 in range(2):
                kvacc[2 * gprev + g2] += _dot_nt(_b(va_r[g2]), ph[g2])
        if g is not None:
            v = _dot(_b(wkv[pl.ds(r0 + 72, 72), :]), xt)
            for g2 in range(2):
                va_w[g2] = _u(jnp.concatenate([v[72 * g2:72 * g2 + 72], ones8], axis=0).astype(bf16))
            if side is not None:
                for n in range(4):
                    side(4 + n, token(v, n))

    pkb1[...] = jnp.zeros_like(pkb1)
    vab1[...] = jnp.zeros_like(vab1)

    def a1_block(j, carry, rel):
        for jb in ((2, 3) if rel else (1,)):
            @pl.when(j == jb)
            def _():
                start_batch(jb)
        cp_xa(j).wait()
        if rel:
            for q in range(4):
                cp_w(j - 2, q).wait()
        for q in range(4):
            a1_step(j, q, (q + 3) % 4, q % 2, functools.partial(relayout, j - 2, q) if rel else None)
        return carry
    lax.fori_loop(0, 2, functools.partial(a1_block, rel=False), 0)
    lax.fori_loop(2, 4, functools.partial(a1_block, rel=True), 0)

    def xtrans(gidx):
        c0 = pl.multiple_of(gidx * 128, 128)
        xnat[pl.ds(c0, 128), :] = _b(xbt[:, pl.ds(c0, 128)]).astype(f32).T

    cp_waq.wait()
    cp_woa.wait()
    cp_xb0.wait()
    cp_mem.wait()
    r3 = _iota((72, 80), 0)
    c3 = _iota((72, 80), 1)
    pw = [jnp.where(c3 - 8 * g2 == (r3 & 3) * AD + (r3 >> 2), 1.0, 0.0).astype(bf16) for g2 in range(2)]
    def prep_wo(g):
        y = jnp.concatenate(
            [_dot(pw[g2], _b(woa[72 * g + 32 * g2:72 * g + 32 * g2 + 40, :])) for g2 in range(2)], axis=0)
        wop[72 * g:72 * g + 72, :] = _u(y.astype(bf16))
        return y

    def prep_q(g):
        y = fold2(g, 0, 0, pc)
        wqt[72 * g:72 * g + 72, :] = _u(y.astype(bf16))
        return y

    def pq_early(g, j):
        y = _dot(_b(wqt[72 * g:72 * g + 72, :]), _b(xat[:, 512 * j:512 * j + 512]))
        pqb[GR * g:GR * g + GR, 512 * j:512 * j + 512] = y
        return y

    def wo_trans(n):
        w = min(128, DM - 128 * n)
        wopt[64 * n:64 * n + w // 2, :] = _u(_b(wop[:, 128 * n:128 * n + w]).T)

    for qs, jobs in (((0, 1), [("w", g) for g in range(G)] + [("q", g) for g in range(NE)]
                      + [("e", (g, j)) for g in range(NE) for j in range(4)]),
                     ((2, 3), [("q", g) for g in range(NE, G)])):
        for q in qs:
            cp_w(2, q).wait()
        toks = []
        for k, (kind, arg) in enumerate(jobs):
            y = prep_wo(arg) if kind == "w" else prep_q(arg) if kind == "q" else pq_early(*arg)
            toks += [token(y, n) for n in range(4)]
            if qs[0] == 0 and k == 1:
                a1_step(None, None, 3, 0)
        for n in range(16):
            relayout(2, qs[n // 8], n % 8, toks[n * len(toks) // 16])
        for n in ((0, 1, 2) if qs[0] == 0 else (3, 4)):
            wo_trans(n)
    r4 = _iota((80, GR), 0)
    c4 = _iota((80, GR), 1)
    for g in range(2 * G):
        kvt[g] = _u(jnp.where((r4 & 3) == (c4 & 3), kvacc[g], 0.0).astype(bf16))
    xtrans(0)
    xtrans(1)
    ri = _iota((80, 80), 0)
    ci = _iota((80, 80), 1)
    same = (ri < 40) == (ci < 40)
    valid = same & (((ri >= 32) & (ri < 48)) | ((ci >= 32) & (ci < 48)) | (ci <= ri))
    fill[...] = jnp.where(valid, 0.0, jnp.where(same, -1e9 / SCALE, -jnp.inf)).astype(f32)

    def W(c0, n):
        return _b(wqkv[:, pl.ds(c0, n)])

    def WO(r0, n):
        return _b(wo32[r0 // 2:(r0 + n) // 2, :])

    def wot_rem(h):
        r0 = h * (DM // 2) + 256
        return _b(wot[pl.ds(r0 if isinstance(r0, int) else pl.multiple_of(r0, 8), 32), :])

    def tails(p):
        return jnp.concatenate(
            [xnat[pl.ds(pl.multiple_of(128 * p + 32 * c + 24, 8), 8), :] for c in range(4)], axis=0)

    lhs0 = jnp.concatenate([tails(0), xnat[0:32, :]], axis=0).astype(bf16)

    def pro(i, c):
        for k in range(PU):
            cp_wo(PU * i + k).wait()
        for k in range(PU):
            c0 = pl.multiple_of((PU * i + k) * 768, 128)
            y = _dot(lhs0, W(c0, 768))
            ringB[0, :, pl.ds(c0, 768)] = y[0:32]
            A0[0:24, pl.ds(c0, 768)] = y[32:56]
            for hh in range(2):
                h = 2 * (PU * i + k) + hh
                blk = _b(wot[pl.ds(pl.multiple_of(h * (DM // 2), 8), 256), :])
                wo32[pl.ds(pl.multiple_of(h * 64, 64), 64), :] = _u(blk.T)
            rem = jnp.concatenate([wot_rem(2 * (PU * i + k)), wot_rem(2 * (PU * i + k) + 1)], axis=0)
            wor[PU * i + k] = _u(rem.T)
        return c
    lax.fori_loop(0, NP // PU, pro, 0)

    def out_copy(gidx):
        r0 = pl.multiple_of(gidx * 128, 128)
        return pltpu.make_async_copy(outb.at[pl.ds(r0, 128), :], out_h.at[pl.ds(r0, 128), :], sem_out.at[gidx])

    def period(p, mem):
        pn = jnp.minimum(p + 1, NPER - 1)
        pcur = p % 2
        pnx = 1 - pcur
        xo = tails(pn).astype(bf16)
        xt = _b(xat[:, pl.ds(pl.multiple_of(p * 128, 128), 128)])
        st = {"rt": None}

        st["ph"] = {}

        def a2_pq(gs):
            for g in gs:
                if g < NE:
                    st["ph"][g] = _features(pqb[GR * g:GR * g + GR, pl.ds(pl.multiple_of(p * 128, 128), 128)])
                else:
                    st["ph"][g] = _features(_dot(_b(wqt[72 * g:72 * g + 72, :]), xt))

        def a2_num():
            os_ = []
            for g in range(2 * G):
                nd = _dot(_b(kvt[g]), st["ph"][g // 2][g % 2])
                rden = 1.0 / (nd[72:80] + 1e-6)
                os_.append((nd[0:72].reshape(9, 8, 128) * rden[None]).reshape(72, 128))
            st["oa"] = jnp.concatenate(os_, axis=0).astype(bf16)

        def a2_out():
            y = jnp.concatenate([_dot(_b(wopt[72 * g:72 * g + 72, :]), st["oa"]) for g in range(G)], axis=0)
            outb[pl.ds(pl.multiple_of(p * 128, 128), 128), 0:DM] = y.T.astype(bf16)

        a_stage = (lambda: a2_pq((1, 2, 3)), lambda: a2_pq((0,)), a2_num, a2_out)

        for r in range(4):
            Ac, An = (A0, A1) if r % 2 == 0 else (A1, A0)
            t = 4 * p + r
            tn = jnp.minimum(t + 1, 4 * NPER - 1)
            xn = xnat[pl.ds(pl.multiple_of(32 * tn, 32), 24), :]
            lhs = jnp.concatenate([mem, xn], axis=0).astype(bf16)
            fl = fill[...]
            Ac[24:32, :] = ringB[pcur, 8 * r:8 * r + 8, :]
            ys, ps, os_ = {}, {}, {}
            acc = [None, None]

            def st_qkv(i):
                y = _dot(lhs, W(768 * i, 768))
                An[0:24, 768 * i:768 * (i + 1)] = y[8:32]
                ys[i] = y[0:8]

            def gather(i, ym, o1):
                c1 = 768 * i + o1
                o2 = o1 + 384
                return jnp.concatenate([Ac[:, c1:c1 + 128], ym[:, o1:o1 + 128], ym[:, o2:o2 + 128],
                                        Ac[:, c1 + 384:c1 + 512]], axis=0).astype(bf16)

            def st_qk(i):
                s = _dot_nt(gather(i, ys[i], 0), gather(i, ys[i], 128))
                s = jnp.where(fl == 0.0, s, fl)
                m = jnp.max(s, axis=-1, keepdims=True)
                e = jnp.exp2((s - m) * (SCALE * LOG2E))
                ps[i] = (e.astype(bf16), jnp.sum(e, axis=-1, keepdims=True))

            def st_pv(i):
                e, l = ps.pop(i)
                os_[i] = _dot(e, gather(i, ys.pop(i), 256)) * (1.0 / l)

            def st_o(i):
                o = os_.pop(i)
                om, ox = (o[32:40], o[40:48]), (o[0:32], o[48:80])
                cols = [slice(256 * i + 128 * hh, 256 * i + 128 * hh + 128) for hh in range(2)]
                if r % 2 == 0:
                    lo = [jnp.concatenate([om[hh], ox[hh][0:24]], axis=0) for hh in range(2)]
                    for hh in range(2):
                        odef[:, cols[hh]] = ox[hh][24:32]
                else:
                    lo = [jnp.concatenate([om[hh], odef[:, cols[hh]], ox[hh]], axis=0) for hh in range(2)]
                y = _dot(jnp.concatenate(lo, axis=1).astype(bf16), WO(256 * i, 256))
                acc[0] = y if acc[0] is None else acc[0] + y
                y = _dot(o[32:48].astype(bf16), _b(wor[i]))
                acc[1] = y if acc[1] is None else acc[1] + y
                oxb = jnp.concatenate(ox, axis=1).astype(bf16)
                if r < 3:
                    obuf[16 * r:16 * r + 16, 256 * i:256 * i + 256] = _u(oxb)
                else:
                    blk = jnp.concatenate([_b(obuf[:, 256 * i:256 * i + 256]), oxb], axis=0)
                    y = _dot_nt(jnp.concatenate([wot_rem(2 * i), wot_rem(2 * i + 1)], axis=1), blk)
                    st["rt"] = y if st["rt"] is None else st["rt"] + y

            def f_xqkv(j):
                c0 = r * 3072 + 768 * j
                ringB[pnx, :, c0:c0 + 768] = _dot(xo, W(c0, 768))

            for i in range(NP + 4):
                if i < NP:
                    st_qkv(i)
                else:
                    if r in (1, 2) and i == NP + 3:
                        a_stage[r]()
                    f_xqkv(i - NP)
                    if r in (0, 3) and i == NP + 1:
                        a_stage[r]()
                if 0 <= i - 1 < NP:
                    st_qk(i - 1)
                if 0 <= i - 2 < NP:
                    st_pv(i - 2)
                if 0 <= i - 3 < NP:
                    st_o(i - 3)
            assert not os_ and not ps and not ys
            if r % 2 == 0:
                outb[pl.ds(pl.multiple_of(32 * t, 32), 24), DM:DM + 512] = acc[0][8:32].astype(bf16)
            else:
                outb[pl.ds(pl.multiple_of(32 * t - 8, 8), 40), DM:DM + 512] = acc[0][8:48].astype(bf16)
            mrem = acc[1][0:8] + pltpu.roll(acc[1][8:16], 64, 1)
            mem = jnp.concatenate([acc[0][0:8], mrem[:, 0:64]], axis=1)

        rt = jnp.concatenate([jnp.zeros((64, 128), f32), st["rt"]], axis=0).T
        outb[pl.ds(pl.multiple_of(p * 128, 128), 128), DM + 512:2 * DM] = rt[:, 64:128].astype(bf16)
        xtrans(jnp.minimum(p + 2, NPER - 1))
        out_copy(p).start()

        @pl.when(p == 0)
        def _():
            cp_xb1.wait()
        return mem

    lax.fori_loop(0, nper, period, mem0[...].astype(f32))
    for gidx in range(nper):
        out_copy(gidx).wait()


def build(nper=NPER):
    V = pltpu.VMEM
    scratch = [
        V((DM // 2, S), u32),
        V((DM // 2, 3 * DM), u32),
        V((AD, AD, AH), bf16),
        V((DM // 2, DM), u32),
        V((DM // 2, S), u32),
        V((M, DM), bf16),
        V((3 * H, DM // 2, E), u32),
        V((H * DM // 2, E), u32),
        V((32, 640), f32),
        V((DM, DM), u32),
        V((DM // 2, DM), u32),
        V((DM // 2, DM), u32),
        V((DM // 2, DM), u32),
        V((2 * G, 80, GR), f32),
        V((2 * G, 40, GR), u32),
        V((NE * GR, S), f32),
        V((GR, 512), f32),
        V((GR, 512), f32),
        V((2, 40, 512), u32),
        V((2, 40, 512), u32),
        V((DM // 2, 3 * H * E), u32),
        V((H * E // 2, 512), u32),
        V((NP, 64, E), u32),
        V((S, DM), f32),
        V((32, 3 * H * E), f32),
        V((32, 3 * H * E), f32),
        V((2, 32, 3 * H * E), f32),
        V((8, H * E), f32),
        V((48, H * E), u32),
        V((80, 80), f32),
        V((S, 2 * DM), bf16),
        pltpu.SemaphoreType.DMA((8 + 4 + 12 + NP,)),
        pltpu.SemaphoreType.DMA((NPER,)),
    ]

    def fn(A_x, A_wqkv, A_w_phi, A_wo, B_x, B_mem0, B_Wq, B_Wk, B_Wv, B_Wo):
        out = pl.pallas_call(
            functools.partial(_kernel, nper=nper),
            out_shape=jax.ShapeDtypeStruct((S, 2 * DM), bf16),
            in_specs=[pl.BlockSpec(memory_space=pl.ANY)] * 10,
            out_specs=pl.BlockSpec(memory_space=pl.ANY),
            scratch_shapes=scratch,
            compiler_params=pltpu.CompilerParams(vmem_limit_bytes=104 * 1024 * 1024),
        )(
            jnp.swapaxes(A_x, 1, 2).reshape(DM, S),
            A_wqkv,
            jnp.transpose(A_w_phi, (1, 2, 0)),
            A_wo,
            jnp.swapaxes(B_x, 1, 2).reshape(DM, S),
            B_mem0.reshape(M, DM),
            B_Wq.reshape(DM // 2, 2 * H, E),
            B_Wk.reshape(DM // 2, 2 * H, E),
            B_Wv.reshape(DM // 2, 2 * H, E),
            jnp.swapaxes(B_Wo, 1, 2).reshape(H * DM, E),
        )
        return out.reshape(1, S, 2 * DM)
    return fn


_impl = jax.jit(build())


def pallas_concat_heads__linear_kernel_hedgehog__memory_aug_recurrent_mem_tr__prompt_kernel(
    A_x, A_wqkv, A_w_phi, A_wo, B_x, B_mem0, B_Wq, B_Wk, B_Wv, B_Wo, B_seg_len,
):
    if isinstance(B_seg_len, int):
        assert B_seg_len == SEG
    assert A_x.shape == (1, S, DM) and B_x.shape == (1, S, DM) and B_mem0.shape == (1, M, DM)
    return _impl(A_x, A_wqkv, A_w_phi, A_wo, B_x, B_mem0, B_Wq, B_Wk, B_Wv, B_Wo)
```

```python
import functools
import jax
import jax.numpy as jnp
from jax import lax
from jax.experimental import pallas as pl
from jax.experimental.pallas import tpu as pltpu

f32, bf16, u32, i32 = jnp.float32, jnp.bfloat16, jnp.uint32, jnp.int32

S, DM = 2048, 576
H, E, M, SEG = 32, 128, 8, 32
NP = H // 2
NPER = S // (4 * SEG)
AH, AD = 32, 18
G, GR = 4, 144
NE = 1
PU = 2
NT = 2
SCALE = float(E) ** -0.5
LOG2E = 1.4426950408889634


def _dot(a, b):
    return jnp.dot(a, b, preferred_element_type=f32)


def _dot_nt(a, b):
    return lax.dot_general(a, b, (((1,), (1,)), ((), ())), preferred_element_type=f32)


def _b(x):
    return pltpu.bitcast(x, bf16)


def _u(x):
    return pltpu.bitcast(x, u32)


def _iota(shape, dim):
    return lax.broadcasted_iota(i32, shape, dim)


def _features(p):
    t = p.shape[1]
    outs = []
    for g2 in range(2):
        x3 = p[72 * g2:72 * g2 + 72].reshape(9, 8, t)
        mx = jnp.max(x3, axis=0)
        mx = jnp.maximum(mx, pltpu.roll(mx, 4, 0))
        mn = jnp.min(x3, axis=0)
        mn = jnp.minimum(mn, pltpu.roll(mn, 4, 0))
        ep = jnp.exp(x3 - mx[None])
        en = jnp.exp(mn[None] - x3)
        sp = jnp.sum(ep, axis=0)
        sn = jnp.sum(en, axis=0)
        rp = 1.0 / (sp + pltpu.roll(sp, 4, 0))
        rn = 1.0 / (sn + pltpu.roll(sn, 4, 0))
        phi = jnp.concatenate([ep * rp[None], en * rn[None]], axis=0)
        outs.append(phi.reshape(GR, t).astype(bf16))
    return outs


def _kernel(xat_h, wa_h, phi_h, woa_h, xbt_h, mem_h, wq_h, wk_h, wv_h, wot_h, out_h,
            xat, wa, phi, woa, xbt, mem0, wst, wot,
            pc, wkv, wqt, wop, wopt, kvacc, kvt, pqb, pkb0, pkb1, vab0, vab1,
            wqkv, wo32, wor, xnat, A0, A1, ringB, odef, obuf, fill, outb,
            sem_in, sem_out, *, nper):
    xat_h, wa_h, woa_h, xbt_h, wot_h = [r.bitcast(u32) for r in (xat_h, wa_h, woa_h, xbt_h, wot_h)]
    cp_phi = pltpu.make_async_copy(phi_h, phi, sem_in.at[0])
    cp_wak = pltpu.make_async_copy(wa_h.at[:, 512:1152], wa.at[:, 512:1152], sem_in.at[1])
    cp_wav = pltpu.make_async_copy(wa_h.at[:, 1152:1728], wa.at[:, 1152:1728], sem_in.at[2])
    cp_waq = pltpu.make_async_copy(wa_h.at[:, 0:512], wa.at[:, 0:512], sem_in.at[3])
    cp_woa = pltpu.make_async_copy(woa_h, woa, sem_in.at[4])
    cp_mem = pltpu.make_async_copy(mem_h, mem0, sem_in.at[5])
    cp_xb0 = pltpu.make_async_copy(xbt_h.at[:, 0:384], xbt.at[:, 0:384], sem_in.at[6])
    cp_xb1 = pltpu.make_async_copy(xbt_h.at[:, 384:S], xbt.at[:, 384:S], sem_in.at[7])

    def cp_xa(c):
        cols = pl.ds(pl.multiple_of(c * 512, 512), 512)
        return pltpu.make_async_copy(xat_h.at[:, cols], xat.at[:, cols], sem_in.at[8 + c])

    def start_w(which, q):
        src = (wq_h, wk_h, wv_h)[which].bitcast(u32)
        for jj in range(4):
            for par in range(2):
                pltpu.make_async_copy(src.at[:, par * 16 + 4 * q + jj, :],
                                      wst.at[which * 32 + q * 8 + jj * 2 + par],
                                      sem_in.at[12 + which * 4 + q]).start()

    def cp_w(which, q):
        chunk = wst.at[pl.ds(which * 32 + q * 8, 8)]
        return pltpu.make_async_copy(chunk, chunk, sem_in.at[12 + which * 4 + q])

    def cp_wo(i):
        rows = pl.ds(pl.multiple_of(i * DM, DM), DM)
        return pltpu.make_async_copy(wot_h.at[rows, :], wot.at[rows, :], sem_in.at[24 + i])

    cp_phi.start()
    cp_wak.start()
    cp_wav.start()
    cp_xa(0).start()

    def start_batch(n):
        if n < 3:
            cp_xa(1 + n).start()
            if n == 2:
                cp_waq.start()
                cp_woa.start()
                cp_xb0.start()
                cp_mem.start()
            for q in range(4):
                start_w(n, q)
        else:
            for i in range(NP):
                cp_wo(i).start()
            cp_xb1.start()
    start_batch(0)

    pc[...] = jnp.zeros_like(pc)
    kvacc[...] = jnp.zeros_like(kvacc)
    row = _iota((DM, 640), 0)
    col = _iota((DM, 640), 1)
    perm = jnp.where(col == (row & 31) * AD + (row >> 5), 1.0, 0.0).astype(bf16)
    cp_phi.wait()
    for d in range(AD):
        pc[0:AD, 32 * d:32 * d + 32] = phi[d].astype(f32)
    rt = _dot(pc[:, 0:DM].astype(bf16), perm)
    pc[...] = rt
    rtk = pltpu.roll(rt, 64, 1)

    def window(hg, shift):
        lo = shift + 72 * hg
        c0 = lo // 128 * 128
        return c0, min((lo + 71) // 128 * 128 + 128, shift + DM) - c0

    def fold(hg, shift, base, src):
        c0, n = window(hg, shift)
        r2 = _iota((72, n), 0)
        rel = _iota((72, n), 1) + (c0 - shift - 72 * hg) - (r2 & 3) * AD
        if src is None:
            sel = jnp.where(rel == (r2 >> 2), 1.0, 0.0)
        else:
            w = jnp.broadcast_to(src[0:AD, c0:c0 + n][:, None, :], (AD, 8, n)).reshape(9, 2, 8, n)
            w = jnp.where(_iota((9, 8, n), 1) < 4, w[:, 0], w[:, 1]).reshape(72, n)
            sel = jnp.where((rel >= 0) & (rel < AD), w, 0.0)
        return _dot_nt(sel.astype(bf16), _b(wa[:, base + c0:base + c0 + n]))

    def fold2(g, shift, base, src):
        return jnp.concatenate([fold(2 * g, shift, base, src), fold(2 * g + 1, shift, base, src)], axis=0)

    cp_wak.wait()
    for g in range(G):
        wkv[GR * g:GR * g + 72, :] = _u(fold2(g, 64, 512, rtk).astype(bf16))
    cp_wav.wait()
    for g in range(G):
        wkv[GR * g + 72:GR * g + 144, :] = _u(fold2(g, 0, 1152, None).astype(bf16))

    ones8 = jnp.ones((8, 512), f32)

    def relayout(which, q, piece, tok):
        jj, half = piece // 2, piece % 2
        c0 = pl.multiple_of((4 * q + jj) * 768 + which * 128, 128)
        for k in range(NT):
            n = GR // NT
            rows = pl.ds(half * GR + k * n, n)
            ev = wst[which * 32 + q * 8 + jj * 2, rows, :].reshape(n // 8, 8, E) | tok[k][None]
            od = wst[which * 32 + q * 8 + jj * 2 + 1, rows, :].reshape(n // 8, 8, E) | tok[k][None]
            wqkv[rows, pl.ds(c0, 128)] = ((ev & u32(0xFFFF)) | (od << 16)).reshape(n, E)
            wqkv[rows, pl.ds(c0 + 384, 128)] = ((ev >> 16) | (od & u32(0xFFFF0000))).reshape(n, E)

    def token(y, n):
        out = []
        for k in range(NT):
            r = (GR // NT) * k
            bits = pltpu.bitcast(y[r:r + 8, 128 * n:128 * n + 128], u32)
            out.append(bits & (bits + 1) & 1)
        return out

    def a1_step(j, g, gprev, par, side=None):
        pk_w, pk_r = (pkb0, pkb1) if par == 0 else (pkb1, pkb0)
        va_w, va_r = (vab0, vab1) if par == 0 else (vab1, vab0)
        if g is not None:
            xt = _b(xat[:, pl.ds(pl.multiple_of(512 * j, 512), 512)])
            r0 = g * GR
            pk = _dot(_b(wkv[pl.ds(r0, 72), :]), xt)
            pk_w[...] = pk
            if side is not None:
                for n in range(4):
                    side(n, token(pk, n))
        if gprev is not None:
            ph = _features(pk_r[...])
            for g2 in range(2):
                kvacc[2 * gprev + g2] += _dot_nt(_b(va_r[g2]), ph[g2])
        if g is not None:
            v = _dot(_b(wkv[pl.ds(r0 + 72, 72), :]), xt)
            for g2 in range(2):
                va_w[g2] = _u(jnp.concatenate([v[72 * g2:72 * g2 + 72], ones8], axis=0).astype(bf16))
            if side is not None:
                for n in range(4):
                    side(4 + n, token(v, n))

    pkb1[...] = jnp.zeros_like(pkb1)
    vab1[...] = jnp.zeros_like(vab1)

    def a1_block(j, carry, rel):
        for jb in ((2, 3) if rel else (1,)):
            @pl.when(j == jb)
            def _():
                start_batch(jb)
        cp_xa(j).wait()
        if rel:
            for q in range(4):
                cp_w(j - 2, q).wait()
        for q in range(4):
            a1_step(j, q, (q + 3) % 4, q % 2, functools.partial(relayout, j - 2, q) if rel else None)
        return carry
    lax.fori_loop(0, 2, functools.partial(a1_block, rel=False), 0)
    lax.fori_loop(2, 4, functools.partial(a1_block, rel=True), 0)

    def xtrans(gidx):
        c0 = pl.multiple_of(gidx * 128, 128)
        xnat[pl.ds(c0, 128), :] = _b(xbt[:, pl.ds(c0, 128)]).astype(f32).T

    cp_waq.wait()
    cp_woa.wait()
    cp_xb0.wait()
    cp_mem.wait()
    r3 = _iota((72, 80), 0)
    c3 = _iota((72, 80), 1)
    pw = [jnp.where(c3 - 8 * g2 == (r3 & 3) * AD + (r3 >> 2), 1.0, 0.0).astype(bf16) for g2 in range(2)]
    def prep_wo(g):
        y = jnp.concatenate(
            [_dot(pw[g2], _b(woa[72 * g + 32 * g2:72 * g + 32 * g2 + 40, :])) for g2 in range(2)], axis=0)
        wop[72 * g:72 * g + 72, :] = _u(y.astype(bf16))
        return y

    def prep_q(g):
        y = fold2(g, 0, 0, pc)
        wqt[72 * g:72 * g + 72, :] = _u(y.astype(bf16))
        return y

    def pq_early(g, j):
        y = _dot(_b(wqt[72 * g:72 * g + 72, :]), _b(xat[:, 512 * j:512 * j + 512]))
        pqb[GR * g:GR * g + GR, 512 * j:512 * j + 512] = y
        return y

    def wo_trans(n):
        w = min(128, DM - 128 * n)
        wopt[64 * n:64 * n + w // 2, :] = _u(_b(wop[:, 128 * n:128 * n + w]).T)

    for qs, jobs in (((0, 1), [("w", g) for g in range(G)] + [("q", g) for g in range(NE)]
                      + [("e", (g, j)) for g in range(NE) for j in range(4)]),
                     ((2, 3), [("q", g) for g in range(NE, G)])):
        for q in qs:
            cp_w(2, q).wait()
        toks = []
        for k, (kind, arg) in enumerate(jobs):
            y = prep_wo(arg) if kind == "w" else prep_q(arg) if kind == "q" else pq_early(*arg)
            toks += [token(y, n) for n in range(4)]
            if qs[0] == 0 and k == 1:
                a1_step(None, None, 3, 0)
        for n in range(16):
            relayout(2, qs[n // 8], n % 8, toks[n * len(toks) // 16])
        for n in ((0, 1, 2) if qs[0] == 0 else (3, 4)):
            wo_trans(n)
    r4 = _iota((80, GR), 0)
    c4 = _iota((80, GR), 1)
    for g in range(2 * G):
        kvt[g] = _u(jnp.where((r4 & 3) == (c4 & 3), kvacc[g], 0.0).astype(bf16))
    xtrans(0)
    xtrans(1)
    ri = _iota((80, 80), 0)
    ci = _iota((80, 80), 1)
    same = (ri < 40) == (ci < 40)
    valid = same & (((ri >= 32) & (ri < 48)) | ((ci >= 32) & (ci < 48)) | (ci <= ri))
    fill[...] = jnp.where(valid, 0.0, jnp.where(same, -1e9 / SCALE, -jnp.inf)).astype(f32)

    def W(c0, n):
        return _b(wqkv[:, pl.ds(c0, n)])

    def WO(r0, n):
        return _b(wo32[r0 // 2:(r0 + n) // 2, :])

    def wot_rem(h):
        r0 = h * (DM // 2) + 256
        return _b(wot[pl.ds(r0 if isinstance(r0, int) else pl.multiple_of(r0, 8), 32), :])

    def tails(p):
        return jnp.concatenate(
            [xnat[pl.ds(pl.multiple_of(128 * p + 32 * c + 24, 8), 8), :] for c in range(4)], axis=0)

    lhs0 = jnp.concatenate([tails(0), xnat[0:32, :]], axis=0).astype(bf16)

    def pro(i, c):
        for k in range(PU):
            cp_wo(PU * i + k).wait()
        for k in range(PU):
            c0 = pl.multiple_of((PU * i + k) * 768, 128)
            y = _dot(lhs0, W(c0, 768))
            ringB[0, :, pl.ds(c0, 768)] = y[0:32]
            A0[0:24, pl.ds(c0, 768)] = y[32:56]
            for hh in range(2):
                h = 2 * (PU * i + k) + hh
                blk = _b(wot[pl.ds(pl.multiple_of(h * (DM // 2), 8), 256), :])
                wo32[pl.ds(pl.multiple_of(h * 64, 64), 64), :] = _u(blk.T)
            rem = jnp.concatenate([wot_rem(2 * (PU * i + k)), wot_rem(2 * (PU * i + k) + 1)], axis=0)
            wor[PU * i + k] = _u(rem.T)
        return c
    lax.fori_loop(0, NP // PU, pro, 0)

    def out_copy(gidx):
        r0 = pl.multiple_of(gidx * 128, 128)
        return pltpu.make_async_copy(outb.at[pl.ds(r0, 128), :], out_h.at[pl.ds(r0, 128), :], sem_out.at[gidx])

    def period(p, mem):
        pn = jnp.minimum(p + 1, NPER - 1)
        pcur = p % 2
        pnx = 1 - pcur
        xo = tails(pn).astype(bf16)
        xt = _b(xat[:, pl.ds(pl.multiple_of(p * 128, 128), 128)])
        st = {"rt": None}

        st["ph"] = {}

        def a2_pq(gs):
            for g in gs:
                if g < NE:
                    st["ph"][g] = _features(pqb[GR * g:GR * g + GR, pl.ds(pl.multiple_of(p * 128, 128), 128)])
                else:
                    st["ph"][g] = _features(_dot(_b(wqt[72 * g:72 * g + 72, :]), xt))

        def a2_num():
            os_ = []
            for g in range(2 * G):
                nd = _dot(_b(kvt[g]), st["ph"][g // 2][g % 2])
                rden = 1.0 / (nd[72:80] + 1e-6)
                os_.append((nd[0:72].reshape(9, 8, 128) * rden[None]).reshape(72, 128))
            st["oa"] = jnp.concatenate(os_, axis=0).astype(bf16)

        def a2_out():
            y = jnp.concatenate([_dot(_b(wopt[72 * g:72 * g + 72, :]), st["oa"]) for g in range(G)], axis=0)
            outb[pl.ds(pl.multiple_of(p * 128, 128), 128), 0:DM] = y.T.astype(bf16)

        a_stage = (lambda: a2_pq((1, 2, 3)), lambda: a2_pq((0,)), a2_num, a2_out)

        for r in range(4):
            Ac, An = (A0, A1) if r % 2 == 0 else (A1, A0)
            t = 4 * p + r
            tn = jnp.minimum(t + 1, 4 * NPER - 1)
            xn = xnat[pl.ds(pl.multiple_of(32 * tn, 32), 24), :]
            lhs = jnp.concatenate([mem, xn], axis=0).astype(bf16)
            fl = fill[...]
            Ac[24:32, :] = ringB[pcur, 8 * r:8 * r + 8, :]
            ys, ps, os_ = {}, {}, {}
            acc = [None, None]

            def st_qkv(i):
                y = _dot(lhs, W(768 * i, 768))
                An[0:24, 768 * i:768 * (i + 1)] = y[8:32]
                ys[i] = y[0:8]

            def gather(i, ym, o1):
                c1 = 768 * i + o1
                o2 = o1 + 384
                return jnp.concatenate([Ac[:, c1:c1 + 128], ym[:, o1:o1 + 128], ym[:, o2:o2 + 128],
                                        Ac[:, c1 + 384:c1 + 512]], axis=0).astype(bf16)

            def st_qk(i):
                s = _dot_nt(gather(i, ys[i], 0), gather(i, ys[i], 128))
                s = jnp.where(fl == 0.0, s, fl)
                m = jnp.max(s, axis=-1, keepdims=True)
                e = jnp.exp2((s - m) * (SCALE * LOG2E))
                ps[i] = (e.astype(bf16), jnp.sum(e, axis=-1, keepdims=True))

            def st_pv(i):
                e, l = ps.pop(i)
                os_[i] = _dot(e, gather(i, ys.pop(i), 256)) * (1.0 / l)

            def st_o(i):
                o = os_[i]
                om, ox = (o[32:40], o[40:48]), (o[0:32], o[48:80])
                cols = [slice(256 * i + 128 * hh, 256 * i + 128 * hh + 128) for hh in range(2)]
                if r % 2 == 0:
                    lo = [jnp.concatenate([om[hh], ox[hh][0:24]], axis=0) for hh in range(2)]
                    for hh in range(2):
                        odef[:, cols[hh]] = ox[hh][24:32]
                else:
                    lo = [jnp.concatenate([om[hh], odef[:, cols[hh]], ox[hh]], axis=0) for hh in range(2)]
                y = _dot(jnp.concatenate(lo, axis=1).astype(bf16), WO(256 * i, 256))
                acc[0] = y if acc[0] is None else acc[0] + y

            def st_r(i):
                y = _dot(os_[i][32:48].astype(bf16), _b(wor[i]))
                acc[1] = y if acc[1] is None else acc[1] + y

            def st_b(i):
                o = os_[i]
                oxb = jnp.concatenate([o[0:32], o[48:80]], axis=1).astype(bf16)
                if r < 3:
                    obuf[16 * r:16 * r + 16, 256 * i:256 * i + 256] = _u(oxb)
                else:
                    blk = jnp.concatenate([_b(obuf[:, 256 * i:256 * i + 256]), oxb], axis=0)
                    y = _dot_nt(jnp.concatenate([wot_rem(2 * i), wot_rem(2 * i + 1)], axis=1), blk)
                    st["rt"] = y if st["rt"] is None else st["rt"] + y

            def f_xqkv(j):
                c0 = r * 3072 + 768 * j
                ringB[pnx, :, c0:c0 + 768] = _dot(xo, W(c0, 768))

            for i in range(NP + 4):
                if i < NP:
                    st_qkv(i)
                else:
                    if r in (1, 2) and i == NP + 3:
                        a_stage[r]()
                    f_xqkv(i - NP)
                    if r in (0, 3) and i == NP + 1:
                        a_stage[r]()
                if 0 <= i - 3 < NP:
                    st_o(i - 3)
                    st_r(i - 3)
                    st_b(i - 3)
                if 0 <= i - 1 < NP:
                    st_qk(i - 1)
                if 0 <= i - 2 < NP:
                    st_pv(i - 2)
            if r % 2 == 0:
                outb[pl.ds(pl.multiple_of(32 * t, 32), 24), DM:DM + 512] = acc[0][8:32].astype(bf16)
            else:
                outb[pl.ds(pl.multiple_of(32 * t - 8, 8), 40), DM:DM + 512] = acc[0][8:48].astype(bf16)
            mrem = acc[1][0:8] + pltpu.roll(acc[1][8:16], 64, 1)
            mem = jnp.concatenate([acc[0][0:8], mrem[:, 0:64]], axis=1)

        rt = jnp.concatenate([jnp.zeros((64, 128), f32), st["rt"]], axis=0).T
        outb[pl.ds(pl.multiple_of(p * 128, 128), 128), DM + 512:2 * DM] = rt[:, 64:128].astype(bf16)
        xtrans(jnp.minimum(p + 2, NPER - 1))
        out_copy(p).start()

        @pl.when(p == 0)
        def _():
            cp_xb1.wait()
        return mem

    lax.fori_loop(0, nper, period, mem0[...].astype(f32))
    for gidx in range(nper):
        out_copy(gidx).wait()


def build(nper=NPER):
    V = pltpu.VMEM
    scratch = [
        V((DM // 2, S), u32),
        V((DM // 2, 3 * DM), u32),
        V((AD, AD, AH), bf16),
        V((DM // 2, DM), u32),
        V((DM // 2, S), u32),
        V((M, DM), bf16),
        V((3 * H, DM // 2, E), u32),
        V((H * DM // 2, E), u32),
        V((32, 640), f32),
        V((DM, DM), u32),
        V((DM // 2, DM), u32),
        V((DM // 2, DM), u32),
        V((DM // 2, DM), u32),
        V((2 * G, 80, GR), f32),
        V((2 * G, 40, GR), u32),
        V((NE * GR, S), f32),
        V((GR, 512), f32),
        V((GR, 512), f32),
        V((2, 40, 512), u32),
        V((2, 40, 512), u32),
        V((DM // 2, 3 * H * E), u32),
        V((H * E // 2, 512), u32),
        V((NP, 64, E), u32),
        V((S, DM), f32),
        V((32, 3 * H * E), f32),
        V((32, 3 * H * E), f32),
        V((2, 32, 3 * H * E), f32),
        V((8, H * E), f32),
        V((48, H * E), u32),
        V((80, 80), f32),
        V((S, 2 * DM), bf16),
        pltpu.SemaphoreType.DMA((8 + 4 + 12 + NP,)),
        pltpu.SemaphoreType.DMA((NPER,)),
    ]

    def fn(A_x, A_wqkv, A_w_phi, A_wo, B_x, B_mem0, B_Wq, B_Wk, B_Wv, B_Wo):
        out = pl.pallas_call(
            functools.partial(_kernel, nper=nper),
            out_shape=jax.ShapeDtypeStruct((S, 2 * DM), bf16),
            in_specs=[pl.BlockSpec(memory_space=pl.ANY)] * 10,
            out_specs=pl.BlockSpec(memory_space=pl.ANY),
            scratch_shapes=scratch,
            compiler_params=pltpu.CompilerParams(vmem_limit_bytes=104 * 1024 * 1024),
        )(
            jnp.swapaxes(A_x, 1, 2).reshape(DM, S),
            A_wqkv,
            jnp.transpose(A_w_phi, (1, 2, 0)),
            A_wo,
            jnp.swapaxes(B_x, 1, 2).reshape(DM, S),
            B_mem0.reshape(M, DM),
            B_Wq.reshape(DM // 2, 2 * H, E),
            B_Wk.reshape(DM // 2, 2 * H, E),
            B_Wv.reshape(DM // 2, 2 * H, E),
            jnp.swapaxes(B_Wo, 1, 2).reshape(H * DM, E),
        )
        return out.reshape(1, S, 2 * DM)
    return fn


_impl = jax.jit(build())


def pallas_concat_heads__linear_kernel_hedgehog__memory_aug_recurrent_mem_tr__prompt_kernel(
    A_x, A_wqkv, A_w_phi, A_wo, B_x, B_mem0, B_Wq, B_Wk, B_Wv, B_Wo, B_seg_len,
):
    if isinstance(B_seg_len, int):
        assert B_seg_len == SEG
    assert A_x.shape == (1, S, DM) and B_x.shape == (1, S, DM) and B_mem0.shape == (1, M, DM)
    return _impl(A_x, A_wqkv, A_w_phi, A_wo, B_x, B_mem0, B_Wq, B_Wk, B_Wv, B_Wo)
```

```python
import functools
import jax
import jax.numpy as jnp
from jax import lax
from jax.experimental import pallas as pl
from jax.experimental.pallas import tpu as pltpu

f32, bf16, u32, i32 = jnp.float32, jnp.bfloat16, jnp.uint32, jnp.int32

S, DM = 2048, 576
H, E, M, SEG = 32, 128, 8, 32
NP = H // 2
NPER = S // (4 * SEG)
AH, AD = 32, 18
G, GR = 4, 144
NE = 1
PU = 2
NT = 2
SCALE = float(E) ** -0.5
LOG2E = 1.4426950408889634


def _dot(a, b):
    return jnp.dot(a, b, preferred_element_type=f32)


def _dot_nt(a, b):
    return lax.dot_general(a, b, (((1,), (1,)), ((), ())), preferred_element_type=f32)


def _b(x):
    return pltpu.bitcast(x, bf16)


def _u(x):
    return pltpu.bitcast(x, u32)


def _iota(shape, dim):
    return lax.broadcasted_iota(i32, shape, dim)


def _features(p):
    t = p.shape[1]
    outs = []
    for g2 in range(2):
        x3 = p[72 * g2:72 * g2 + 72].reshape(9, 8, t)
        mx = jnp.max(x3, axis=0)
        mx = jnp.maximum(mx, pltpu.roll(mx, 4, 0))
        mn = jnp.min(x3, axis=0)
        mn = jnp.minimum(mn, pltpu.roll(mn, 4, 0))
        ep = jnp.exp(x3 - mx[None])
        en = jnp.exp(mn[None] - x3)
        sp = jnp.sum(ep, axis=0)
        sn = jnp.sum(en, axis=0)
        rp = 1.0 / (sp + pltpu.roll(sp, 4, 0))
        rn = 1.0 / (sn + pltpu.roll(sn, 4, 0))
        phi = jnp.concatenate([ep * rp[None], en * rn[None]], axis=0)
        outs.append(phi.reshape(GR, t).astype(bf16))
    return outs


def _kernel(xat_h, wa_h, phi_h, woa_h, xbt_h, mem_h, wq_h, wk_h, wv_h, wot_h, out_h,
            xat, wa, phi, woa, xbt, mem0, wst, wot,
            pc, wkv, wqt, wop, wopt, kvacc, kvt, pqb, pkb0, pkb1, vab0, vab1,
            wqkv, wo32, wor, xnat, A0, A1, ringB, odef, obuf, fill, outb,
            sem_in, sem_out, *, nper):
    xat_h, wa_h, woa_h, xbt_h, wot_h = [r.bitcast(u32) for r in (xat_h, wa_h, woa_h, xbt_h, wot_h)]
    cp_phi = pltpu.make_async_copy(phi_h, phi, sem_in.at[0])
    cp_wak = pltpu.make_async_copy(wa_h.at[:, 512:1152], wa.at[:, 512:1152], sem_in.at[1])
    cp_wav = pltpu.make_async_copy(wa_h.at[:, 1152:1728], wa.at[:, 1152:1728], sem_in.at[2])
    cp_waq = pltpu.make_async_copy(wa_h.at[:, 0:512], wa.at[:, 0:512], sem_in.at[3])
    cp_woa = pltpu.make_async_copy(woa_h, woa, sem_in.at[4])
    cp_mem = pltpu.make_async_copy(mem_h, mem0, sem_in.at[5])
    cp_xb0 = pltpu.make_async_copy(xbt_h.at[:, 0:384], xbt.at[:, 0:384], sem_in.at[6])
    cp_xb1 = pltpu.make_async_copy(xbt_h.at[:, 384:S], xbt.at[:, 384:S], sem_in.at[7])

    def cp_xa(c):
        cols = pl.ds(pl.multiple_of(c * 512, 512), 512)
        return pltpu.make_async_copy(xat_h.at[:, cols], xat.at[:, cols], sem_in.at[8 + c])

    def start_w(which, q):
        src = (wq_h, wk_h, wv_h)[which].bitcast(u32)
        for jj in range(4):
            for par in range(2):
                pltpu.make_async_copy(src.at[:, par * 16 + 4 * q + jj, :],
                                      wst.at[which * 32 + q * 8 + jj * 2 + par],
                                      sem_in.at[12 + which * 4 + q]).start()

    def cp_w(which, q):
        chunk = wst.at[pl.ds(which * 32 + q * 8, 8)]
        return pltpu.make_async_copy(chunk, chunk, sem_in.at[12 + which * 4 + q])

    def cp_wo(i):
        rows = pl.ds(pl.multiple_of(i * DM, DM), DM)
        return pltpu.make_async_copy(wot_h.at[rows, :], wot.at[rows, :], sem_in.at[24 + i])

    cp_phi.start()
    cp_wak.start()
    cp_wav.start()
    cp_xa(0).start()

    def start_batch(n):
        if n < 3:
            cp_xa(1 + n).start()
            if n == 2:
                cp_waq.start()
                cp_woa.start()
                cp_xb0.start()
                cp_mem.start()
            for q in range(4):
                start_w(n, q)
        else:
            for i in range(NP):
                cp_wo(i).start()
            cp_xb1.start()
    start_batch(0)

    pc[...] = jnp.zeros_like(pc)
    kvacc[...] = jnp.zeros_like(kvacc)
    row = _iota((DM, 640), 0)
    col = _iota((DM, 640), 1)
    perm = jnp.where(col == (row & 31) * AD + (row >> 5), 1.0, 0.0).astype(bf16)
    cp_phi.wait()
    for d in range(AD):
        pc[0:AD, 32 * d:32 * d + 32] = phi[d].astype(f32)
    rt = _dot(pc[:, 0:DM].astype(bf16), perm)
    pc[...] = rt
    rtk = pltpu.roll(rt, 64, 1)

    def window(hg, shift):
        lo = shift + 72 * hg
        c0 = lo // 128 * 128
        return c0, min((lo + 71) // 128 * 128 + 128, shift + DM) - c0

    def fold(hg, shift, base, src):
        c0, n = window(hg, shift)
        r2 = _iota((72, n), 0)
        rel = _iota((72, n), 1) + (c0 - shift - 72 * hg) - (r2 & 3) * AD
        if src is None:
            sel = jnp.where(rel == (r2 >> 2), 1.0, 0.0)
        else:
            w = jnp.broadcast_to(src[0:AD, c0:c0 + n][:, None, :], (AD, 8, n)).reshape(9, 2, 8, n)
            w = jnp.where(_iota((9, 8, n), 1) < 4, w[:, 0], w[:, 1]).reshape(72, n)
            sel = jnp.where((rel >= 0) & (rel < AD), w, 0.0)
        return _dot_nt(sel.astype(bf16), _b(wa[:, base + c0:base + c0 + n]))

    def fold2(g, shift, base, src):
        return jnp.concatenate([fold(2 * g, shift, base, src), fold(2 * g + 1, shift, base, src)], axis=0)

    cp_wak.wait()
    for g in range(G):
        wkv[GR * g:GR * g + 72, :] = _u(fold2(g, 64, 512, rtk).astype(bf16))
    cp_wav.wait()
    for g in range(G):
        wkv[GR * g + 72:GR * g + 144, :] = _u(fold2(g, 0, 1152, None).astype(bf16))

    ones8 = jnp.ones((8, 512), f32)

    def relayout(which, q, piece, tok):
        jj, half = piece // 2, piece % 2
        c0 = pl.multiple_of((4 * q + jj) * 768 + which * 128, 128)
        for k in range(NT):
            n = GR // NT
            rows = pl.ds(half * GR + k * n, n)
            ev = wst[which * 32 + q * 8 + jj * 2, rows, :].reshape(n // 8, 8, E) | tok[k][None]
            od = wst[which * 32 + q * 8 + jj * 2 + 1, rows, :].reshape(n // 8, 8, E) | tok[k][None]
            wqkv[rows, pl.ds(c0, 128)] = ((ev & u32(0xFFFF)) | (od << 16)).reshape(n, E)
            wqkv[rows, pl.ds(c0 + 384, 128)] = ((ev >> 16) | (od & u32(0xFFFF0000))).reshape(n, E)

    def token(y, n):
        out = []
        for k in range(NT):
            r = (GR // NT) * k
            bits = pltpu.bitcast(y[r:r + 8, 128 * n:128 * n + 128], u32)
            out.append(bits & (bits + 1) & 1)
        return out

    def a1_step(j, g, gprev, par, side=None):
        pk_w, pk_r = (pkb0, pkb1) if par == 0 else (pkb1, pkb0)
        va_w, va_r = (vab0, vab1) if par == 0 else (vab1, vab0)
        if g is not None:
            xt = _b(xat[:, pl.ds(pl.multiple_of(512 * j, 512), 512)])
            r0 = g * GR
            pk = _dot(_b(wkv[pl.ds(r0, 72), :]), xt)
            pk_w[...] = pk
            if side is not None:
                for n in range(4):
                    side(n, token(pk, n))
        if gprev is not None:
            ph = _features(pk_r[...])
            for g2 in range(2):
                kvacc[2 * gprev + g2] += _dot_nt(_b(va_r[g2]), ph[g2])
        if g is not None:
            v = _dot(_b(wkv[pl.ds(r0 + 72, 72), :]), xt)
            for g2 in range(2):
                va_w[g2] = _u(jnp.concatenate([v[72 * g2:72 * g2 + 72], ones8], axis=0).astype(bf16))
            if side is not None:
                for n in range(4):
                    side(4 + n, token(v, n))

    pkb1[...] = jnp.zeros_like(pkb1)
    vab1[...] = jnp.zeros_like(vab1)

    def a1_block(j, carry, rel):
        for jb in ((2, 3) if rel else (1,)):
            @pl.when(j == jb)
            def _():
                start_batch(jb)
        cp_xa(j).wait()
        if rel:
            for q in range(4):
                cp_w(j - 2, q).wait()
        for q in range(4):
            a1_step(j, q, (q + 3) % 4, q % 2, functools.partial(relayout, j - 2, q) if rel else None)
        return carry
    lax.fori_loop(0, 2, functools.partial(a1_block, rel=False), 0)
    lax.fori_loop(2, 4, functools.partial(a1_block, rel=True), 0)

    def xtrans(gidx):
        c0 = pl.multiple_of(gidx * 128, 128)
        xnat[pl.ds(c0, 128), :] = _b(xbt[:, pl.ds(c0, 128)]).astype(f32).T

    cp_waq.wait()
    cp_woa.wait()
    cp_xb0.wait()
    cp_mem.wait()
    r3 = _iota((72, 80), 0)
    c3 = _iota((72, 80), 1)
    pw = [jnp.where(c3 - 8 * g2 == (r3 & 3) * AD + (r3 >> 2), 1.0, 0.0).astype(bf16) for g2 in range(2)]

    def prep_wo(g):
        y = jnp.concatenate(
            [_dot(pw[g2], _b(woa[72 * g + 32 * g2:72 * g + 32 * g2 + 40, :])) for g2 in range(2)], axis=0)
        wop[72 * g:72 * g + 72, :] = _u(y.astype(bf16))
        return y

    def prep_q(g):
        y = fold2(g, 0, 0, pc)
        wqt[72 * g:72 * g + 72, :] = _u(y.astype(bf16))
        return y

    def pq_early(g, j):
        y = _dot(_b(wqt[72 * g:72 * g + 72, :]), _b(xat[:, 512 * j:512 * j + 512]))
        pqb[GR * g:GR * g + GR, 512 * j:512 * j + 512] = y
        return y

    def wo_trans(n):
        w = min(128, DM - 128 * n)
        wopt[64 * n:64 * n + w // 2, :] = _u(_b(wop[:, 128 * n:128 * n + w]).T)

    def misc():
        r4 = _iota((80, GR), 0)
        c4 = _iota((80, GR), 1)
        for g in range(2 * G):
            kvt[g] = _u(jnp.where((r4 & 3) == (c4 & 3), kvacc[g], 0.0).astype(bf16))
        xtrans(0)
        xtrans(1)
        ri = _iota((80, 80), 0)
        ci = _iota((80, 80), 1)
        same = (ri < 40) == (ci < 40)
        valid = same & (((ri >= 32) & (ri < 48)) | ((ci >= 32) & (ci < 48)) | (ci <= ri))
        fill[...] = jnp.where(valid, 0.0, jnp.where(same, -1e9 / SCALE, -jnp.inf)).astype(f32)

    for qs, jobs in (((0, 1), [("w", g) for g in range(G)] + [("q", g) for g in range(NE)]
                      + [("e", (g, j)) for g in range(NE) for j in range(4)]),
                     ((2, 3), [("q", g) for g in range(NE, G)])):
        for q in qs:
            cp_w(2, q).wait()
        toks = []
        for k, (kind, arg) in enumerate(jobs):
            y = prep_wo(arg) if kind == "w" else prep_q(arg) if kind == "q" else pq_early(*arg)
            toks += [token(y, n) for n in range(4)]
            if qs[0] == 0 and k == 1:
                a1_step(None, None, 3, 0)
        for n in range(16):
            relayout(2, qs[n // 8], n % 8, toks[n * len(toks) // 16])
        for n in ((0, 1, 2) if qs[0] == 0 else (3, 4)):
            wo_trans(n)
        if qs[0] == 0:
            misc()

    def W(c0, n):
        return _b(wqkv[:, pl.ds(c0, n)])

    def WO(r0, n):
        return _b(wo32[r0 // 2:(r0 + n) // 2, :])

    def wot_rem(h):
        r0 = h * (DM // 2) + 256
        return _b(wot[pl.ds(r0 if isinstance(r0, int) else pl.multiple_of(r0, 8), 32), :])

    def tails(p):
        return jnp.concatenate(
            [xnat[pl.ds(pl.multiple_of(128 * p + 32 * c + 24, 8), 8), :] for c in range(4)], axis=0)

    lhs0 = jnp.concatenate([tails(0), xnat[0:32, :]], axis=0).astype(bf16)

    def pro(i, c):
        for k in range(PU):
            cp_wo(PU * i + k).wait()
        for k in range(PU):
            c0 = pl.multiple_of((PU * i + k) * 768, 128)
            y = _dot(lhs0, W(c0, 768))
            ringB[0, :, pl.ds(c0, 768)] = y[0:32]
            A0[0:24, pl.ds(c0, 768)] = y[32:56]
            for hh in range(2):
                h = 2 * (PU * i + k) + hh
                blk = _b(wot[pl.ds(pl.multiple_of(h * (DM // 2), 8), 256), :])
                wo32[pl.ds(pl.multiple_of(h * 64, 64), 64), :] = _u(blk.T)
            rem = jnp.concatenate([wot_rem(2 * (PU * i + k)), wot_rem(2 * (PU * i + k) + 1)], axis=0)
            wor[PU * i + k] = _u(rem.T)
        return c
    lax.fori_loop(0, NP // PU, pro, 0)

    def out_copy(gidx):
        r0 = pl.multiple_of(gidx * 128, 128)
        return pltpu.make_async_copy(outb.at[pl.ds(r0, 128), :], out_h.at[pl.ds(r0, 128), :], sem_out.at[gidx])

    def period(p, mem):
        pn = jnp.minimum(p + 1, NPER - 1)
        pcur = p % 2
        pnx = 1 - pcur
        xo = tails(pn).astype(bf16)
        xt = _b(xat[:, pl.ds(pl.multiple_of(p * 128, 128), 128)])
        st = {"rt": None}

        st["ph"] = {}

        def a2_pq(gs):
            for g in gs:
                if g < NE:
                    st["ph"][g] = _features(pqb[GR * g:GR * g + GR, pl.ds(pl.multiple_of(p * 128, 128), 128)])
                else:
                    st["ph"][g] = _features(_dot(_b(wqt[72 * g:72 * g + 72, :]), xt))

        def a2_num():
            os_ = []
            for g in range(2 * G):
                nd = _dot(_b(kvt[g]), st["ph"][g // 2][g % 2])
                rden = 1.0 / (nd[72:80] + 1e-6)
                os_.append((nd[0:72].reshape(9, 8, 128) * rden[None]).reshape(72, 128))
            st["oa"] = jnp.concatenate(os_, axis=0).astype(bf16)

        def a2_out():
            y = jnp.concatenate([_dot(_b(wopt[72 * g:72 * g + 72, :]), st["oa"]) for g in range(G)], axis=0)
            outb[pl.ds(pl.multiple_of(p * 128, 128), 128), 0:DM] = y.T.astype(bf16)

        a_stage = (lambda: a2_pq((1, 2, 3)), lambda: a2_pq((0,)), a2_num, a2_out)

        for r in range(4):
            Ac, An = (A0, A1) if r % 2 == 0 else (A1, A0)
            t = 4 * p + r
            tn = jnp.minimum(t + 1, 4 * NPER - 1)
            xn = xnat[pl.ds(pl.multiple_of(32 * tn, 32), 24), :]
            lhs = jnp.concatenate([mem, xn], axis=0).astype(bf16)
            fl = fill[...]
            Ac[24:32, :] = ringB[pcur, 8 * r:8 * r + 8, :]
            ys, ps, os_ = {}, {}, {}
            acc = [None, None]

            def st_qkv(i):
                y = _dot(lhs, W(768 * i, 768))
                An[0:24, 768 * i:768 * (i + 1)] = y[8:32]
                ys[i] = y[0:8]

            def gather(i, ym, o1):
                c1 = 768 * i + o1
                o2 = o1 + 384
                return jnp.concatenate([Ac[:, c1:c1 + 128], ym[:, o1:o1 + 128], ym[:, o2:o2 + 128],
                                        Ac[:, c1 + 384:c1 + 512]], axis=0).astype(bf16)

            def st_qk(i):
                s = _dot_nt(gather(i, ys[i], 0), gather(i, ys[i], 128))
                s = jnp.where(fl == 0.0, s, fl)
                m = jnp.max(s, axis=-1, keepdims=True)
                e = jnp.exp2((s - m) * (SCALE * LOG2E))
                ps[i] = (e.astype(bf16), jnp.sum(e, axis=-1, keepdims=True))

            def st_pv(i):
                e, l = ps.pop(i)
                os_[i] = _dot(e, gather(i, ys.pop(i), 256)) * (1.0 / l)

            def st_o(i):
                o = os_[i]
                om, ox = (o[32:40], o[40:48]), (o[0:32], o[48:80])
                cols = [slice(256 * i + 128 * hh, 256 * i + 128 * hh + 128) for hh in range(2)]
                if r % 2 == 0:
                    lo = [jnp.concatenate([om[hh], ox[hh][0:24]], axis=0) for hh in range(2)]
                    for hh in range(2):
                        odef[:, cols[hh]] = ox[hh][24:32]
                else:
                    lo = [jnp.concatenate([om[hh], odef[:, cols[hh]], ox[hh]], axis=0) for hh in range(2)]
                y = _dot(jnp.concatenate(lo, axis=1).astype(bf16), WO(256 * i, 256))
                acc[0] = y if acc[0] is None else acc[0] + y

            def st_r(i):
                y = _dot(os_[i][32:48].astype(bf16), _b(wor[i]))
                acc[1] = y if acc[1] is None else acc[1] + y

            def st_b(i):
                o = os_[i]
                oxb = jnp.concatenate([o[0:32], o[48:80]], axis=1).astype(bf16)
                if r < 3:
                    obuf[16 * r:16 * r + 16, 256 * i:256 * i + 256] = _u(oxb)
                else:
                    blk = jnp.concatenate([_b(obuf[:, 256 * i:256 * i + 256]), oxb], axis=0)
                    y = _dot_nt(jnp.concatenate([wot_rem(2 * i), wot_rem(2 * i + 1)], axis=1), blk)
                    st["rt"] = y if st["rt"] is None else st["rt"] + y

            def f_xqkv(j):
                c0 = r * 3072 + 768 * j
                ringB[pnx, :, c0:c0 + 768] = _dot(xo, W(c0, 768))

            for i in range(NP + 4):
                if i < NP:
                    st_qkv(i)
                else:
                    if r in (1, 2) and i == NP + 3:
                        a_stage[r]()
                    f_xqkv(i - NP)
                    if r in (0, 3) and i == NP + 1:
                        a_stage[r]()
                if 0 <= i - 3 < NP:
                    st_o(i - 3)
                    st_r(i - 3)
                    st_b(i - 3)
                if 0 <= i - 1 < NP:
                    st_qk(i - 1)
                if 0 <= i - 2 < NP:
                    st_pv(i - 2)
            if r % 2 == 0:
                outb[pl.ds(pl.multiple_of(32 * t, 32), 24), DM:DM + 512] = acc[0][8:32].astype(bf16)
            else:
                outb[pl.ds(pl.multiple_of(32 * t - 8, 8), 40), DM:DM + 512] = acc[0][8:48].astype(bf16)
            mrem = acc[1][0:8] + pltpu.roll(acc[1][8:16], 64, 1)
            mem = jnp.concatenate([acc[0][0:8], mrem[:, 0:64]], axis=1)

        rt = jnp.concatenate([jnp.zeros((64, 128), f32), st["rt"]], axis=0).T
        outb[pl.ds(pl.multiple_of(p * 128, 128), 128), DM + 512:2 * DM] = rt[:, 64:128].astype(bf16)
        xtrans(jnp.minimum(p + 2, NPER - 1))
        out_copy(p).start()

        @pl.when(p == 0)
        def _():
            cp_xb1.wait()
        return mem

    lax.fori_loop(0, nper, period, mem0[...].astype(f32))
    for gidx in range(nper):
        out_copy(gidx).wait()


def build(nper=NPER):
    V = pltpu.VMEM
    scratch = [
        V((DM // 2, S), u32),
        V((DM // 2, 3 * DM), u32),
        V((AD, AD, AH), bf16),
        V((DM // 2, DM), u32),
        V((DM // 2, S), u32),
        V((M, DM), bf16),
        V((3 * H, DM // 2, E), u32),
        V((H * DM // 2, E), u32),
        V((32, 640), f32),
        V((DM, DM), u32),
        V((DM // 2, DM), u32),
        V((DM // 2, DM), u32),
        V((DM // 2, DM), u32),
        V((2 * G, 80, GR), f32),
        V((2 * G, 40, GR), u32),
        V((NE * GR, S), f32),
        V((GR, 512), f32),
        V((GR, 512), f32),
        V((2, 40, 512), u32),
        V((2, 40, 512), u32),
        V((DM // 2, 3 * H * E), u32),
        V((H * E // 2, 512), u32),
        V((NP, 64, E), u32),
        V((S, DM), f32),
        V((32, 3 * H * E), f32),
        V((32, 3 * H * E), f32),
        V((2, 32, 3 * H * E), f32),
        V((8, H * E), f32),
        V((48, H * E), u32),
        V((80, 80), f32),
        V((S, 2 * DM), bf16),
        pltpu.SemaphoreType.DMA((8 + 4 + 12 + NP,)),
        pltpu.SemaphoreType.DMA((NPER,)),
    ]

    def fn(A_x, A_wqkv, A_w_phi, A_wo, B_x, B_mem0, B_Wq, B_Wk, B_Wv, B_Wo):
        out = pl.pallas_call(
            functools.partial(_kernel, nper=nper),
            out_shape=jax.ShapeDtypeStruct((S, 2 * DM), bf16),
            in_specs=[pl.BlockSpec(memory_space=pl.ANY)] * 10,
            out_specs=pl.BlockSpec(memory_space=pl.ANY),
            scratch_shapes=scratch,
            compiler_params=pltpu.CompilerParams(vmem_limit_bytes=104 * 1024 * 1024),
        )(
            jnp.swapaxes(A_x, 1, 2).reshape(DM, S),
            A_wqkv,
            jnp.transpose(A_w_phi, (1, 2, 0)),
            A_wo,
            jnp.swapaxes(B_x, 1, 2).reshape(DM, S),
            B_mem0.reshape(M, DM),
            B_Wq.reshape(DM // 2, 2 * H, E),
            B_Wk.reshape(DM // 2, 2 * H, E),
            B_Wv.reshape(DM // 2, 2 * H, E),
            jnp.swapaxes(B_Wo, 1, 2).reshape(H * DM, E),
        )
        return out.reshape(1, S, 2 * DM)
    return fn


_impl = jax.jit(build())


def pallas_concat_heads__linear_kernel_hedgehog__memory_aug_recurrent_mem_tr__prompt_kernel(
    A_x, A_wqkv, A_w_phi, A_wo, B_x, B_mem0, B_Wq, B_Wk, B_Wv, B_Wo, B_seg_len,
):
    if isinstance(B_seg_len, int):
        assert B_seg_len == SEG
    assert A_x.shape == (1, S, DM) and B_x.shape == (1, S, DM) and B_mem0.shape == (1, M, DM)
    return _impl(A_x, A_wqkv, A_w_phi, A_wo, B_x, B_mem0, B_Wq, B_Wk, B_Wv, B_Wo)
```
